```python
import jax
import jax.numpy as jnp

def _softmax(x, axis=-1):
    return jax.nn.softmax(x, axis=axis)
def _gelu(x):
    return jax.nn.gelu(x, approximate=True)
def _silu(x):
    return jax.nn.silu(x)
def _sigmoid(x):
    return jax.nn.sigmoid(x)
def _layernorm(x, axis=-1, eps=1e-5):
    m = jnp.mean(x, axis=axis, keepdims=True)
    v = jnp.var(x, axis=axis, keepdims=True)
    return (x - m) / jnp.sqrt(v + eps)
def _scatter_add(tgt, idx, src, axis=0):
    return tgt.at[idx].add(src)
def _segment_sum(src, seg, n):
    return jax.ops.segment_sum(src, seg, n)
class _Rng:
    def __init__(self, key):
        self._k = key
    def _next(self):
        self._k, sub = jax.random.split(self._k)
        return sub
    def normal(self, shape):
        return jax.random.normal(self._next(), shape, dtype=jnp.bfloat16)
    def randint(self, lo, hi, shape):
        return jax.random.randint(self._next(), shape, lo, hi, dtype=jnp.int32)
    def uniform(self, shape, lo=0.0, hi=1.0):
        return jax.random.uniform(self._next(), shape, jnp.bfloat16, lo, hi)
    def permutation(self, n):
        return jax.random.permutation(self._next(), n)


kernel_name = 'interleave_layers__sliding_block_cached__mixer_s_mlp__decode'

def setup_inputs():
    _rng = _Rng(jax.random.key(int.from_bytes(__import__("os").urandom(4), "little")))
    _w = (lambda a: (lambda t: t.astype(jnp.bfloat16) if jnp.issubdtype(t.dtype, jnp.floating) else t)(jnp.asarray(a)))
    def _A_setup():
        B, Sq, D = 1, 1, 640
        Hq, Hkv, Sk, Dh = 32, 32, 32768, 192
        assert Hq % Hkv == 0, (Hq, Hkv)
        return {
            "x": _w((lambda *s: _rng.normal(s) * 0.05)(B, Sq, D)),
            "k_cache": _w((lambda *s: _rng.normal(s) * 0.05)(B, Hkv, Sk, Dh)),
            "v_cache": _w((lambda *s: _rng.normal(s) * 0.05)(B, Hkv, Sk, Dh)),
            "wq": _w((lambda *s: _rng.normal(s) * 0.05)(D, Hq * Dh) * (D ** -0.5)),
            "wo": _w((lambda *s: _rng.normal(s) * 0.05)(Hq * Dh, D) * ((Hq * Dh) ** -0.5)),
        }
    _A_in = _A_setup()

    def _B_setup():
        B, S, D, F = 1, 1, 640, 1536
        return {
            "x":  _w((lambda *s: _rng.normal(s) * 0.05)(B, S, D)),
            "w1": _w((lambda *s: _rng.normal(s) * 0.05)(D, D) * (D ** -0.5)),
            "w2": _w((lambda *s: _rng.normal(s) * 0.05)(D, D) * (D ** -0.5)),
            "w3": _w((lambda *s: _rng.normal(s) * 0.05)(D, F) * (D ** -0.5)),
            "w4": _w((lambda *s: _rng.normal(s) * 0.05)(F, D) * (F ** -0.5)),
        }
    _B_in = _B_setup()

    return {
        "A_x": _A_in["x"],
        "A_k_cache": _A_in["k_cache"],
        "A_v_cache": _A_in["v_cache"],
        "A_wq": _A_in["wq"],
        "A_wo": _A_in["wo"],
        "B_x": _B_in["x"],
        "B_w1": _B_in["w1"],
        "B_w2": _B_in["w2"],
        "B_w3": _B_in["w3"],
        "B_w4": _B_in["w4"],
    }

def reference(A_x, A_k_cache, A_v_cache, A_wq, A_wo, B_x, B_w1, B_w2, B_w3, B_w4):
    def _A_ref(x, k_cache, v_cache, wq, wo):
        B, Sq, D = x.shape
        Hq, Dh = 32, 192
        Hkv, Sk = k_cache.shape[1], k_cache.shape[2]
        W = min(4096, max(256, Sk // 4))
        rep = Hq // Hkv
        q = (lambda x, *d: x.transpose(*d))((x @ wq).reshape(B, Sq, Hq, Dh), 0, 2, 1, 3)
        k = jnp.repeat(k_cache[:, :, Sk - W:, :], rep, axis=1)
        v = jnp.repeat(v_cache[:, :, Sk - W:, :], rep, axis=1)
        scores = jnp.einsum("bhqd,bhkd->bhqk", q, k) * (Dh ** -0.5)
        p = _softmax(scores, axis=-1)
        o = jnp.einsum("bhqk,bhkd->bhqd", p, v)
        return (lambda x, *d: x.transpose(*d))(o, 0, 2, 1, 3).reshape(B, Sq, Hq * Dh) @ wo

    def _B_ref(x, w1, w2, w3, w4):
        B, S, D = x.shape
        h = _gelu(_layernorm(x, axis=-1) @ w1)
        c = D // 4
        g0 = jnp.pad(h[:, :, 0*c:1*c], ((0, 0), (1, 0), (0, 0)))[:, :S, :]
        g1 = jnp.pad(h[:, :, 1*c:2*c], ((0, 0), (0, 1), (0, 0)))[:, 1:, :]
        g2 = jnp.pad(h[:, :, 2*c:3*c], ((0, 0), (2, 0), (0, 0)))[:, :S, :]
        g3 = jnp.pad(h[:, :, 3*c:   ], ((0, 0), (0, 2), (0, 0)))[:, 2:, :]
        hs = jnp.concatenate([g0, g1, g2, g3], axis=-1) @ w2
        x1 = x + hs
        h2 = _gelu(_layernorm(x1, axis=-1) @ w3) @ w4
        return x1 + h2

    x = A_x
    x = x + _A_ref(_layernorm(x, axis=-1), A_k_cache, A_v_cache, A_wq, A_wo)
    x = x + _B_ref(_layernorm(x, axis=-1), B_w1, B_w2, B_w3, B_w4)
    x = x + _A_ref(_layernorm(x, axis=-1), A_k_cache, A_v_cache, A_wq, A_wo)
    x = x + _B_ref(_layernorm(x, axis=-1), B_w1, B_w2, B_w3, B_w4)
    return x
```

```python
import functools

import jax
import jax.numpy as jnp
from jax import lax
import jax.experimental.pallas as pl
import jax.experimental.pallas.tpu as pltpu

F32 = jnp.float32
BF16 = jnp.bfloat16

_HQ = 32
_DH = 192
_NH = 4
_EPS = 1e-5


def _tile_view(w):
    r, c = w.shape
    return w.reshape(r // 16, 2, 8, c // 128, 128).transpose(0, 1, 3, 2, 4)


def _layernorm(x):
    m = jnp.mean(x, axis=-1, keepdims=True)
    xc = x - m
    v = jnp.mean(xc * xc, axis=-1, keepdims=True)
    return xc * lax.rsqrt(v + _EPS)


def _kernel(x_ref, k_hbm, v_hbm, wq_hbm, wo_hbm, w3_hbm, w4_hbm, o_ref,
            kbuf, vbuf, wqb, wob, w3b, w4b, q_sc, sem_k, sem_v, sem_o, sem_w,
            *, st0, nst):
    ng = _HQ // _NH
    rg = _NH * _DH // 16
    gw = _NH * _DH
    d_model = x_ref.shape[-1]
    d_ff = w3b.shape[1] * 128

    def retile_copies(src, dst, rows, cols, sem):
        return [
            pltpu.make_async_copy(src.at[rows, a, cols],
                                  dst.at[rows, :, pl.ds(8 * a, 8), :], sem)
            for a in range(2)
        ]

    def full(n):
        return pl.ds(0, n)

    def wait_total(dst, sem):
        pltpu.make_async_copy(dst, dst, sem).wait()

    copies = retile_copies(wq_hbm, wqb, full(wqb.shape[0]), full(wqb.shape[1]), sem_w.at[0])
    for g in range(ng):
        rows = pl.ds(g * rg, rg)
        copies += retile_copies(k_hbm, kbuf, rows, pl.ds(st0, nst), sem_k.at[g])
        copies += retile_copies(v_hbm, vbuf, rows, pl.ds(st0, nst), sem_v.at[g])
        copies += retile_copies(wo_hbm, wob, rows, full(wob.shape[1]), sem_o.at[g])
    copies += retile_copies(w3_hbm, w3b, full(w3b.shape[0]), full(w3b.shape[1]), sem_w.at[1])
    copies += retile_copies(w4_hbm, w4b, full(w4b.shape[0]), full(w4b.shape[1]), sem_w.at[2])
    for c in copies:
        c.start()

    def matvec(lhs, wbuf, rows=None):
        kdim = lhs.shape[1]
        cols = []
        for ct in range(wbuf.shape[1]):
            w = wbuf[:, ct] if rows is None else wbuf[rows, ct]
            cols.append(w.reshape(kdim, 128))
        return jnp.dot(lhs, jnp.concatenate(cols, axis=1), preferred_element_type=F32)

    row_id = lax.broadcasted_iota(jnp.int32, (8, gw), 0)
    lane_id = lax.broadcasted_iota(jnp.int32, (8, gw), 1)
    head_mask = (lane_id >= row_id * _DH) & (lane_id < (row_id + 1) * _DH)

    def attention(x, first):
        y8 = jnp.broadcast_to(_layernorm(x), (8, d_model)).astype(BF16)
        if first:
            wait_total(wqb, sem_w.at[0])
        q = matvec(y8, wqb) * (_DH ** -0.5)
        for g in range(ng):
            q_sc[g] = jnp.where(head_mask, q[:, g * gw:(g + 1) * gw], 0.0).astype(BF16)

        def group(g, acc):
            rows = pl.ds(g * rg, rg)
            if first:
                wait_total(kbuf.at[rows], sem_k.at[g])
            s = matvec(q_sc[g], kbuf, rows)
            m = jnp.max(s, axis=1, keepdims=True)
            p = jnp.exp(s - m)
            l = jnp.sum(p, axis=1, keepdims=True)
            pb = p.astype(BF16)
            if first:
                wait_total(vbuf.at[rows], sem_v.at[g])
            v = jnp.concatenate([vbuf[rows, st].reshape(gw, 128) for st in range(nst)], axis=1)
            o = lax.dot_general(pb, v, (((1,), (1,)), ((), ())), preferred_element_type=F32)
            o = jnp.where(head_mask, o / l, 0.0).astype(BF16)
            if first:
                wait_total(wob.at[rows], sem_o.at[g])
            return acc + matvec(o, wob, rows)

        acc = lax.fori_loop(0, ng, group, jnp.zeros((8, d_model), F32))
        return jnp.sum(acc, axis=0, keepdims=True)

    def mixer(x, first):
        y = _layernorm(x)
        z8 = jnp.broadcast_to(_layernorm(y), (8, d_model)).astype(BF16)
        if first:
            wait_total(w3b, sem_w.at[1])
        h = jax.nn.gelu(matvec(z8, w3b), approximate=True).astype(BF16)
        if first:
            wait_total(w4b, sem_w.at[2])
        h2 = matvec(h, w4b)
        return y + h2[0:1]

    x = x_ref[...].astype(F32)
    with jax.named_scope("attn1"):
        x = x + attention(x, True)
    with jax.named_scope("mix1"):
        x = x + mixer(x, True)
    with jax.named_scope("attn2"):
        x = x + attention(x, False)
    with jax.named_scope("mix2"):
        x = x + mixer(x, False)
    o_ref[...] = x.astype(o_ref.dtype)


@jax.jit
def pallas_interleave_layers__sliding_block_cached__mixer_s_mlp__decode_kernel(
    A_x: jax.Array,
    A_k_cache: jax.Array,
    A_v_cache: jax.Array,
    A_wq: jax.Array,
    A_wo: jax.Array,
    B_x: jax.Array,
    B_w1: jax.Array,
    B_w2: jax.Array,
    B_w3: jax.Array,
    B_w4: jax.Array,
):
    b, sq, d_model = A_x.shape
    _, hkv, sk, dh = A_k_cache.shape
    assert b == 1 and sq == 1 and hkv == _HQ and dh == _DH
    win = min(4096, max(256, sk // 4))
    assert win % 128 == 0 and (sk - win) % 128 == 0
    nst = win // 128
    st0 = (sk - win) // 128
    d_ff = B_w3.shape[1]

    kt = _tile_view(jnp.swapaxes(A_k_cache, 2, 3).reshape(hkv * dh, sk))
    vt = _tile_view(jnp.swapaxes(A_v_cache, 2, 3).reshape(hkv * dh, sk))
    ng = _HQ // _NH

    out = pl.pallas_call(
        functools.partial(_kernel, st0=st0, nst=nst),
        out_shape=jax.ShapeDtypeStruct((1, d_model), A_x.dtype),
        in_specs=[pl.BlockSpec(memory_space=pltpu.VMEM)]
        + [pl.BlockSpec(memory_space=pl.ANY)] * 6,
        out_specs=pl.BlockSpec(memory_space=pltpu.VMEM),
        scratch_shapes=[
            pltpu.VMEM((hkv * dh // 16, nst, 16, 128), BF16),
            pltpu.VMEM((hkv * dh // 16, nst, 16, 128), BF16),
            pltpu.VMEM((d_model // 16, _HQ * dh // 128, 16, 128), BF16),
            pltpu.VMEM((_HQ * dh // 16, d_model // 128, 16, 128), BF16),
            pltpu.VMEM((d_model // 16, d_ff // 128, 16, 128), BF16),
            pltpu.VMEM((d_ff // 16, d_model // 128, 16, 128), BF16),
            pltpu.VMEM((ng, 8, _NH * dh), BF16),
            pltpu.SemaphoreType.DMA((ng,)),
            pltpu.SemaphoreType.DMA((ng,)),
            pltpu.SemaphoreType.DMA((ng,)),
            pltpu.SemaphoreType.DMA((3,)),
        ],
        compiler_params=pltpu.CompilerParams(vmem_limit_bytes=127 * 1024 * 1024),
        name="interleave_decode",
    )(A_x.reshape(1, d_model), kt, vt, _tile_view(A_wq), _tile_view(A_wo),
      _tile_view(B_w3), _tile_view(B_w4))
    return out.reshape(b, sq, d_model)
```

```python
import functools
import os

import jax
import jax.numpy as jnp
from jax import lax
import jax.experimental.pallas as pl
import jax.experimental.pallas.tpu as pltpu

F32 = jnp.float32
BF16 = jnp.bfloat16
U32 = jnp.uint32

_HQ = 32
_DH = 192
_EPS = 1e-5
_LOG2E = 1.4426950408889634
_UW = 2 * _DH
_NU = _HQ // 2
_KT = _UW // 128
_GU = 2
_NA = 4

_E = os.environ.get
_LAG = int(_E("LAG", 180))
_MINT = int(_E("MINT", 200))
_XM = int(_E("XM", 1))
_XP = int(_E("XP", 2))
_XL = int(_E("XL", 15))
_BLK = int(_E("BLK", 3))
_TC = float(_E("TC", 31))
_VC = float(_E("VC", 1.6))
_SMLAT = int(_E("SMLAT", 200))
_RTOK = int(_E("RTOK", 550))
_TOKS = int(_E("TOKS", 1))
_LOOP = int(_E("LOOP", 1))
_ORD = _E("ORD", "sqxo")
_LEAD = int(_E("LEAD", 0))
_REV = int(_E("REV", 0))
_RPT = int(_E("RPT", 4))
_REV0 = int(_E("REV0", 0))
_REVT = int(_E("REVT", 5))
_CLN = float(_E("CLN", 0))
_CL0 = float(_E("CL0", 16))
_W4C = [int(t) for t in _E("W4C", "8,3,1").split(",")]
_MRG = int(_E("MRG", 1))
_ORDL = _E("ORDL", "xo")


def _bf(x):
    return pltpu.bitcast(x, BF16)


def _dot(a, b):
    return jnp.dot(a, b, preferred_element_type=F32)


def _dot_nt(a, b):
    return lax.dot_general(a, b, (((1,), (1,)), ((), ())), preferred_element_type=F32)


def _iota(shape, axis):
    return lax.broadcasted_iota(jnp.int32, shape, axis)


def _rows16(x8):
    return jnp.concatenate([x8, jnp.zeros_like(x8)], axis=0).astype(BF16)


def _cols(i):
    return slice(i * 128, (i + 1) * 128)


def _layernorm(x):
    m = jnp.mean(x, axis=-1, keepdims=True)
    xc = x - m
    v = jnp.mean(xc * xc, axis=-1, keepdims=True)
    return xc * lax.rsqrt(v + _EPS)


def _center(x):
    xc = x - jnp.mean(x, axis=-1, keepdims=True)
    v = jnp.mean(xc * xc, axis=-1, keepdims=True)
    return xc, v


def _kernel(x_hbm, k_hbm, v_hbm, wq_hbm, wo_hbm, w3_hbm, w4_hbm, o_ref,
            kbuf, vbuf, wqb, wob, w3b, w4b, x_ref,
            qa_sc, qb_sc, pa_sc, pb_sc, acca_sc, accb_sc, oxa_sc, oxb_sc, la_sc, lb_sc,
            y_sc, qs_sc, out_sc, zero_sc,
            sem_k, sem_v, sem_o, sem_q, sem_w, *, s0, win):
    ng = _NU // _GU
    gw = _GU * _UW
    d_model = x_ref.shape[-1]
    d_ff = w3b.shape[1]
    nst = win // 128
    nj = nst // _NA
    nct = d_model // 128
    q_sc, p_sc = (qa_sc, qb_sc), (pa_sc, pb_sc)
    acc_sc, ox_sc, l_sc = (acca_sc, accb_sc), (oxa_sc, oxb_sc), (la_sc, lb_sc)

    kb16, vb16, wq16, wo16, w316, w416 = (
        r.bitcast(BF16) for r in (kbuf, vbuf, wqb, wob, w3b, w4b))

    def k_copy(g):
        us = pl.ds(g * _GU, _GU)
        return pltpu.make_async_copy(k_hbm.at[us, :, pl.ds(s0, win)], kb16.at[us], sem_k.at[g])

    def v_copy(g):
        us = pl.ds(g * _GU, _GU)
        return pltpu.make_async_copy(v_hbm.at[us, :, pl.ds(s0, win)], vb16.at[us], sem_v.at[g])

    def o_copy(g):
        us = pl.ds(g * _GU, _GU)
        return pltpu.make_async_copy(wo_hbm.at[us], wo16.at[us], sem_o.at[g])

    def q_copy(u):
        return pltpu.make_async_copy(wq_hbm.at[:, pl.ds(u * _UW, _UW)], wq16.at[u], sem_q.at[u])

    w3_copy = pltpu.make_async_copy(w3_hbm, w316, sem_w.at[0])
    x_copy = pltpu.make_async_copy(x_hbm, x_ref, sem_w.at[1])
    w4_rows = [(sum(_W4C[:i]) * 128, n * 128) for i, n in enumerate(_W4C)]
    assert sum(_W4C) * 128 == d_ff
    w4_copies = [
        pltpu.make_async_copy(w4_hbm.at[pl.ds(r0, nr)], w416.at[pl.ds(r0, nr)], sem_w.at[2 + i])
        for i, (r0, nr) in enumerate(w4_rows)]

    for g in range(ng):
        k_copy(g).start()
        if g == 0:
            x_copy.start()
        for u in range(g * _GU, (g + 1) * _GU):
            q_copy(u).start()
        v_copy(g).start()
        o_copy(g).start()
    w3_copy.start()
    for c in w4_copies:
        c.start()

    zero_sc[0] = 0
    zero_sc[1] = 0
    for r in (qa_sc, qb_sc, accb_sc, oxa_sc, oxb_sc, out_sc):
        r[...] = jnp.zeros(r.shape, r.dtype)
    lb_sc[...] = jnp.ones(lb_sc.shape, F32)

    scale = _DH ** -0.5

    def attention1(x):
        y16 = jnp.broadcast_to(_layernorm(x), (16, d_model)).astype(BF16)
        y_sc[...] = pltpu.bitcast(y16, U32)

        def group(g, acc):
            row_id, lane_id = _iota((8, gw), 0), _iota((8, gw), 1)
            mask = (lane_id >= row_id * _DH) & (lane_id < (row_id + 1) * _DH)
            us = pl.ds(g * _GU, _GU)
            qs = []
            for i in range(_GU):
                q_copy(g * _GU + i).wait()
                qs.append(_dot(_bf(y_sc[...]), _bf(wqb[g * _GU + i]))[0:8])
            q = _rows16(jnp.where(mask, jnp.concatenate(qs, axis=1) * scale, 0.0))
            k_copy(g).wait()
            s = _dot(q, _bf(kbuf[us].reshape(gw // 2, win)))[0:8]
            m = jnp.max(s, axis=1, keepdims=True)
            p = jnp.exp(s - m)
            l = jnp.sum(p, axis=1, keepdims=True)
            v_copy(g).wait()
            o = _dot_nt(_rows16(p), _bf(vbuf[us].reshape(gw // 2, win)))[0:8]
            o = _rows16(jnp.where(mask, o / l, 0.0))
            o_copy(g).wait()
            return acc + _dot(o, _bf(wob[us].reshape(gw // 2, d_model)))[0:8]

        acc = lax.fori_loop(0, ng, group, jnp.zeros((8, d_model), F32))
        return jnp.sum(acc, axis=0, keepdims=True)

    def attention2(x):
        tile_c = _TC / 4
        zero = zero_sc[0]
        zero2 = zero_sc[1]

        def same_head_reduce(v, op):
            v = op(v, pltpu.roll(v, 4, axis=0))
            return op(v, pltpu.roll(v, 2, axis=0))

        rev = {"q": [], "never": None}
        sclk = {"x": None, "n": 0, "t": 0, "base": None}

        def tick(idx, cycles):
            if not sclk["on"]:
                return idx
            if sclk["x"] is None:
                sclk["x"] = idx + zero
            elif sclk["base"] is not idx:
                sclk["x"] = sclk["x"] + (idx - sclk["base"])
            sclk["base"] = idx
            while sclk["n"] < sclk["t"] - _CL0:
                x = sclk["x"]
                sclk["x"] = (x + zero2) if sclk["n"] % 2 else (x ^ zero2)
                sclk["n"] += 1
            sclk["t"] += cycles
            return sclk["x"]

        def tile_dots(lhs, buf, u, c, ntile):
            t = None
            for k in range(ntile):
                l = lhs[k]
                w = buf[tick(u, _CLN), k * 64:(k + 1) * 64, _cols(c)]
                for _ in range(_RPT):
                    if rev["q"]:
                        l = jnp.where(rev["never"], pltpu.bitcast(rev["q"].pop(0), U32), l)
                d = _dot(_bf(l), _bf(w))[0:8]
                t = d if t is None else t + d
                yield t

        def task_q(u, par):
            odd_row = (_iota((8, _UW), 0) & 1) == 1
            mask = (_iota((8, _UW), 1) >= _DH) == odd_row
            for c in range(_KT):
                yy = [y_sc[:, _cols(k)] for k in range(nct)]
                for t in tile_dots(yy, wqb, u, c, nct):
                    yield tile_c, 0, None
                t = jnp.where(mask[:, _cols(c)], t * qs_sc[...], 0.0)
                w = pltpu.bitcast(jnp.concatenate([t, t], axis=0).astype(BF16), U32)
                for a in range(_NA):
                    pltpu.store(q_sc[par].at[a, :, _cols(c)], w, mask=_iota((8, 128), 0) == a)
                yield 0.0, 0, t

        def task_s(u, par):
            s = [None] * nj
            for a in range(_NA):
                q = [q_sc[par][a, :, _cols(k)] for k in range(_KT)]
                for j in range(nj):
                    for d in tile_dots(q, kbuf, u, a * nj + j, _KT):
                        yield tile_c, 0, None
                    s[j] = d if a == 0 else s[j] + d
                    z = s[j]
                    if a == _NA - 1:
                        z = mrun = s[j] if j == 0 else jnp.maximum(mrun, s[j])
                    yield 0.0, 0, (z if _TOKS and (j + 1) % _TOKS == 0 else None)
            m = jnp.max(same_head_reduce(mrun, jnp.maximum), axis=1, keepdims=True)
            lrun = None
            for j in range(nj):
                p = jnp.exp2(s[j] - m)
                p_sc[par][:, _cols(j)] = p
                lrun = p if lrun is None else lrun + p
            l_sc[par][...] = lrun
            yield 0.0, _SMLAT, lrun

        def task_x(u, par, nx):
            ox = None
            for st in range(nx):
                a, j = divmod(st, nj)
                t = _dot_nt(_rows16(p_sc[par][:, _cols(j)]),
                            _bf(vbuf[tick(u, 2 * _KT * _CLN), :, _cols(st)]))[0:8]
                ox = t if j == 0 else ox + t
                if j == nj - 1 or st == nx - 1:
                    ox_sc[par][a] = ox
                yield 2 * _KT * tile_c, 0, ox[:, (_KT - 1) * 128:]

        def reduce_o(par, nx):
            row, lane = _iota((8, _UW), 0), _iota((8, _UW), 1)
            head_ok = (lane >= _DH) == ((row & 1) == 1)
            l = jnp.sum(same_head_reduce(l_sc[par][...], jnp.add), axis=1, keepdims=True)
            parts = [jnp.sum(acc_sc[par][_cols(c), :].T, axis=0, keepdims=True)
                     for c in range(_KT)]
            o = jnp.concatenate(parts, axis=1)
            if nx:
                o = o + ox_sc[par][0]
            for a in range(1, -(-nx // nj)):
                o = jnp.where(row >= 2 * a, ox_sc[par][a], o)
            nrow = 2 * max(1, -(-nx // nj))
            return jnp.where(head_ok & (row < nrow), o * (1.0 / l), 0.0)

        def task_o(u, o8):
            o16 = [pltpu.bitcast(_rows16(o8[:, _cols(k)]), U32) for k in range(_KT)]
            for c in range(nct):
                for t in tile_dots(o16, wob, u, c, _KT):
                    yield tile_c, 0, None
                t = t + out_sc[:, _cols(c)]
                out_sc[:, _cols(c)] = t
                yield 0.0, 0, t

        def pv_steps(u, par, nx, tokens, never, clock):
            br = 16 * _BLK
            for b in range(_UW // br):
                h = (b * br) // _DH
                acc = None
                for st in range(nx, nst):
                    a, j = divmod(st, nj)
                    r = 2 * a + h
                    pb = jnp.broadcast_to(p_sc[par][r:r + 1, _cols(j)], (8, 128))
                    for z in tokens():
                        pb = jnp.where(never, z, pb)
                    v = _bf(vbuf[u, b * br // 2:(b + 1) * br // 2, _cols(st)]).astype(F32)
                    t = v.reshape(br // 8, 8, 128) * pb[None]
                    acc = t if acc is None else acc + t
                    nrev = _REV0 if clock["v"] < _REVT else _REV
                    if nrev and ((st - nx + 1) % nrev == 0 or st == nst - 1):
                        rev["q"] += [acc[i] for i in range(br // 8)]
                    if st == nst - 1:
                        acc_sc[par][b * br:(b + 1) * br, :] = acc.reshape(br, 128)
                    yield _VC * _BLK

        def chain_gens(*gens):
            for g in gens:
                yield from g

        def stage(u, par, nx, nx_prev, do_s=True, do_q=True, order=_ORD):
            never = _iota((8, 128), 1) < zero
            o8 = reduce_o(1 - par, nx_prev)
            pending = [(_RTOK + 100 * c, o8[:, _cols(c)]) for c in range(_KT)]
            um1 = max(u - 1, 0) if isinstance(u, int) else jnp.maximum(u - 1, 0)
            tasks = {"o": task_o(um1, o8), "x": task_x(u, par, nx)}
            if do_s:
                tasks["s"] = task_s(u + 1, 1 - par)
            if do_q:
                tasks["q"] = task_q(u + 2, par)
            mx = chain_gens(*[tasks[k] for k in order if k in tasks])
            clock = {"v": 0.0, "m": 0.0}

            def tokens():
                ready = [z for (t, z) in pending if t <= clock["v"]]
                pending[:] = [(t, z) for (t, z) in pending if t > clock["v"]]
                return ready

            def mx_until(tv):
                while clock["m"] <= tv:
                    try:
                        cm, lat, z = next(mx)
                    except StopIteration:
                        return
                    clock["m"] += cm
                    if z is not None:
                        pending.append((max(clock["m"] + _LAG + lat, _MINT), z))

            rev["never"] = never
            sclk.update(x=None, n=0, t=0, base=None, on=bool(_CLN))
            mx_until(_LEAD)
            for c in pv_steps(u, par, nx, tokens, never, clock):
                clock["v"] += c
                mx_until(clock["v"] + _LEAD)
            rev["q"] = []
            mx_until(1e9)
            sclk["on"] = False

        def region(tag, fn):
            with jax.named_scope("st%02d" % tag):
                pl.when(zero < tag + 1)(fn)

        sclk["on"] = False
        with jax.named_scope("pro"):
            xc, v = _center(x)
            y_sc[...] = pltpu.bitcast(jnp.broadcast_to(xc, (16, d_model)).astype(BF16), U32)
            qs_sc[...] = jnp.broadcast_to(lax.rsqrt(v + _EPS) * (scale * _LOG2E), (8, 128))
            for _ in chain_gens(task_q(0, 0), task_s(0, 0), task_q(1, 1)):
                pass

        if _LOOP:
            def body(i, c):
                region(0, lambda: stage(2 * i, 0, _XM, _XM))
                region(1, lambda: stage(2 * i + 1, 1, _XM, _XM))
                return c
            lax.fori_loop(0, (_NU - 2) // 2, body, 0)
        else:
            for u in range(_NU - 2):
                region(u, functools.partial(stage, u, u % 2, _XM, _XM))
        region(_NU - 2, lambda: stage(_NU - 2, 0, _XP, _XM, do_q=False))
        last = lambda: stage(_NU - 1, 1, _XL, _XP, do_s=False, do_q=False, order=_ORDL)
        if _MRG:
            last()
        else:
            region(_NU - 1, last)
        for _ in task_o(_NU - 1, reduce_o(1, _XL)):
            pass
        return jnp.sum(out_sc[...], axis=0, keepdims=True)

    def mixer(x, first):
        xc, v = _center(x)
        mc = jnp.mean(xc, axis=-1, keepdims=True)
        r1 = lax.rsqrt(v + _EPS)
        r2 = lax.rsqrt(r1 * r1 * (v - mc * mc) + _EPS)
        row = _iota((16, d_model), 0)
        lhs = jnp.where(row < 8, jnp.broadcast_to(xc, (16, d_model)), 1.0).astype(BF16)
        if first:
            w3_copy.wait()
        h = _dot(lhs, _bf(w3b[...]))
        h = (h[0:8] - mc * h[8:16]) * (r1 * r2)
        h = jax.nn.gelu(h, approximate=True)
        h2 = None
        for i, (r0, nr) in enumerate(w4_rows if first else [(0, d_ff)]):
            if first:
                w4_copies[i].wait()
            t = _dot(_rows16(h[:, r0:r0 + nr]), _bf(w4b[r0 // 2:(r0 + nr) // 2, :]))[0:1]
            h2 = t if h2 is None else h2 + t
        return xc * r1 + h2

    x_copy.wait()
    x = x_ref[...].astype(F32)
    with jax.named_scope("attn1"):
        x = x + attention1(x)
    with jax.named_scope("mix1"):
        x = x + mixer(x, True)
    with jax.named_scope("attn2"):
        x = x + attention2(x)
    with jax.named_scope("mix2"):
        x = x + mixer(x, False)
    o_ref[...] = x.astype(o_ref.dtype)


@jax.jit
def pallas_interleave_layers__sliding_block_cached__mixer_s_mlp__decode_kernel(
    A_x: jax.Array,
    A_k_cache: jax.Array,
    A_v_cache: jax.Array,
    A_wq: jax.Array,
    A_wo: jax.Array,
    B_x: jax.Array,
    B_w1: jax.Array,
    B_w2: jax.Array,
    B_w3: jax.Array,
    B_w4: jax.Array,
):
    b, sq, d_model = A_x.shape
    _, hkv, sk, dh = A_k_cache.shape
    assert b == 1 and sq == 1 and hkv == _HQ and dh == _DH
    win = min(4096, max(256, sk // 4))
    assert win % (128 * _NA) == 0 and (sk - win) % 128 == 0
    d_ff = B_w3.shape[1]

    kt = jnp.swapaxes(A_k_cache, 2, 3).reshape(_NU, _UW, sk)
    vt = jnp.swapaxes(A_v_cache, 2, 3).reshape(_NU, _UW, sk)
    ng = _NU // _GU

    def two(shape, dtype):
        return [pltpu.VMEM(shape, dtype), pltpu.VMEM(shape, dtype)]

    out = pl.pallas_call(
        functools.partial(_kernel, s0=sk - win, win=win),
        out_shape=jax.ShapeDtypeStruct((1, d_model), A_x.dtype),
        in_specs=[pl.BlockSpec(memory_space=pl.ANY)] * 7,
        out_specs=pl.BlockSpec(memory_space=pltpu.VMEM),
        scratch_shapes=[
            pltpu.VMEM((_NU, _UW // 2, win), U32),
            pltpu.VMEM((_NU, _UW // 2, win), U32),
            pltpu.VMEM((_NU, d_model // 2, _UW), U32),
            pltpu.VMEM((_NU, _UW // 2, d_model), U32),
            pltpu.VMEM((d_model // 2, d_ff), U32),
            pltpu.VMEM((d_ff // 2, d_model), U32),
            pltpu.VMEM((1, d_model), A_x.dtype),
            *two((_NA, 8, _UW), U32),
            *two((8, win // _NA), F32),
            *two((_UW, 128), F32),
            *two((_NA, 8, _UW), F32),
            *two((8, 128), F32),
            pltpu.VMEM((8, d_model), U32),
            pltpu.VMEM((8, 128), F32),
            pltpu.VMEM((8, d_model), F32),
            pltpu.SMEM((2,), jnp.int32),
            pltpu.SemaphoreType.DMA((ng,)),
            pltpu.SemaphoreType.DMA((ng,)),
            pltpu.SemaphoreType.DMA((ng,)),
            pltpu.SemaphoreType.DMA((_NU,)),
            pltpu.SemaphoreType.DMA((2 + len(_W4C),)),
        ],
        compiler_params=pltpu.CompilerParams(
            vmem_limit_bytes=127 * 1024 * 1024,
            disable_bounds_checks=True, disable_semaphore_checks=True),
        name="interleave_decode",
    )(A_x.reshape(1, d_model), kt, vt, A_wq, A_wo.reshape(_NU, _UW, d_model), B_w3, B_w4)
    return out.reshape(b, sq, d_model)
```

```python
import functools
import os

import jax
import jax.numpy as jnp
from jax import lax
import jax.experimental.pallas as pl
import jax.experimental.pallas.tpu as pltpu

F32 = jnp.float32
BF16 = jnp.bfloat16
U32 = jnp.uint32

_HQ = 32
_DH = 192
_EPS = 1e-5
_LOG2E = 1.4426950408889634
_UW = 2 * _DH
_NU = _HQ // 2
_KT = _UW // 128
_GU = 2
_NA = 4

_E = os.environ.get
_LAG = int(_E("LAG", 180))
_MINT = int(_E("MINT", 200))
_XM = int(_E("XM", 1))
_XP = int(_E("XP", 2))
_XL = int(_E("XL", 15))
_BLK = int(_E("BLK", 3))
_TC = float(_E("TC", 31))
_VC = float(_E("VC", 1.6))
_SMLAT = int(_E("SMLAT", 200))
_RTOK = int(_E("RTOK", 550))
_TOKS = int(_E("TOKS", 1))
_LOOP = int(_E("LOOP", 1))
_ORD = _E("ORD", "sqxo")
_LEAD = int(_E("LEAD", 0))
_REV = int(_E("REV", 0))
_RPT = int(_E("RPT", 4))
_REV0 = int(_E("REV0", 0))
_REVT = int(_E("REVT", 5))
_CLN = float(_E("CLN", 0))
_CL0 = float(_E("CL0", 16))
_W4C = [int(t) for t in _E("W4C", "8,3,1").split(",")]
_MRG = int(_E("MRG", 1))
_ORDL = _E("ORDL", "xo")


def _bf(x):
    return pltpu.bitcast(x, BF16)


def _tile_view(w):
    *lead, r, c = w.shape
    n = len(lead)
    w = w.reshape(*lead, r // 16, 2, 8, c // 128, 128)
    return w.transpose(*range(n), n, n + 1, n + 3, n + 2, n + 4)


def _mat(x):
    r16, ct = x.shape[0], x.shape[1]
    cols = [x[:, c].reshape(r16 * 8, 128) for c in range(ct)]
    return _bf(cols[0] if ct == 1 else jnp.concatenate(cols, axis=1))


def _dot(a, b):
    return jnp.dot(a, b, preferred_element_type=F32)


def _dot_nt(a, b):
    return lax.dot_general(a, b, (((1,), (1,)), ((), ())), preferred_element_type=F32)


def _iota(shape, axis):
    return lax.broadcasted_iota(jnp.int32, shape, axis)


def _rows16(x8):
    return jnp.concatenate([x8, jnp.zeros_like(x8)], axis=0).astype(BF16)


def _cols(i):
    return slice(i * 128, (i + 1) * 128)


def _layernorm(x):
    m = jnp.mean(x, axis=-1, keepdims=True)
    xc = x - m
    v = jnp.mean(xc * xc, axis=-1, keepdims=True)
    return xc * lax.rsqrt(v + _EPS)


def _center(x):
    xc = x - jnp.mean(x, axis=-1, keepdims=True)
    v = jnp.mean(xc * xc, axis=-1, keepdims=True)
    return xc, v


def _kernel(x_hbm, k_hbm, v_hbm, wq_hbm, wo_hbm, w3_hbm, w4_hbm, o_ref,
            kbuf, vbuf, wqb, wob, w3b, w4b, x_ref,
            qa_sc, qb_sc, pa_sc, pb_sc, acca_sc, accb_sc, oxa_sc, oxb_sc, la_sc, lb_sc,
            y_sc, qs_sc, out_sc, zero_sc,
            sem_k, sem_v, sem_o, sem_w, *, s0, win):
    ng = _NU // _GU
    gw = _GU * _UW
    d_model = x_ref.shape[-1]
    d_ff = w3b.shape[1] * 128
    nst = win // 128
    nj = nst // _NA
    nct = d_model // 128
    q_sc, p_sc = (qa_sc, qb_sc), (pa_sc, pb_sc)
    acc_sc, ox_sc, l_sc = (acca_sc, accb_sc), (oxa_sc, oxb_sc), (la_sc, lb_sc)

    kb16, vb16, wq16, wo16, w316, w416 = (
        r.bitcast(BF16) for r in (kbuf, vbuf, wqb, wob, w3b, w4b))

    class _Retile:
        def __init__(self, src, dst, sem):
            nl = len(dst.shape) - 4
            lead = (slice(None),) * (nl + 1)
            self.copies = [
                pltpu.make_async_copy(
                    src.at[lead + (a,)],
                    dst.at[lead + (slice(None), pl.ds(8 * a, 8))], sem)
                for a in range(2)]

        def start(self):
            for c in self.copies:
                c.start()

        def wait(self):
            for c in self.copies:
                c.wait()

    st0 = s0 // 128

    def k_copy(g):
        us = pl.ds(g * _GU, _GU)
        return _Retile(k_hbm.at[us, :, :, pl.ds(st0, nst)], kb16.at[us], sem_k.at[g])

    def v_copy(g):
        us = pl.ds(g * _GU, _GU)
        return _Retile(v_hbm.at[us, :, :, pl.ds(st0, nst)], vb16.at[us], sem_v.at[g])

    def o_copy(g):
        us = pl.ds(g * _GU, _GU)
        return _Retile(wo_hbm.at[us], wo16.at[us], sem_o.at[g])

    wq_copy = _Retile(wq_hbm, wq16, sem_w.at[0])
    w3_copy = _Retile(w3_hbm, w316, sem_w.at[1])
    x_copy = pltpu.make_async_copy(x_hbm, x_ref, sem_w.at[2])
    w4_rows = [(sum(_W4C[:i]) * 128, n * 128) for i, n in enumerate(_W4C)]
    assert sum(_W4C) * 128 == d_ff
    w4_copies = [
        _Retile(w4_hbm.at[pl.ds(r0 // 16, nr // 16)], w416.at[pl.ds(r0 // 16, nr // 16)],
                sem_w.at[3 + i])
        for i, (r0, nr) in enumerate(w4_rows)]

    wq_copy.start()
    x_copy.start()
    for g in range(ng):
        k_copy(g).start()
        v_copy(g).start()
        o_copy(g).start()
    w3_copy.start()
    for c in w4_copies:
        c.start()

    zero_sc[0] = 0
    zero_sc[1] = 0
    for r in (qa_sc, qb_sc, accb_sc, oxa_sc, oxb_sc, out_sc):
        r[...] = jnp.zeros(r.shape, r.dtype)
    lb_sc[...] = jnp.ones(lb_sc.shape, F32)

    scale = _DH ** -0.5

    def attention1(x):
        y16 = jnp.broadcast_to(_layernorm(x), (16, d_model)).astype(BF16)
        y_sc[...] = pltpu.bitcast(y16, U32)

        wq_copy.wait()

        def group(g, acc):
            row_id, lane_id = _iota((8, gw), 0), _iota((8, gw), 1)
            mask = (lane_id >= row_id * _DH) & (lane_id < (row_id + 1) * _DH)
            us = pl.ds(g * _GU, _GU)
            r16 = gw // 16
            q = _dot(_bf(y_sc[...]), _mat(wqb[:, pl.ds(g * (gw // 128), gw // 128)]))[0:8]
            q = _rows16(jnp.where(mask, q * scale, 0.0))
            k_copy(g).wait()
            s = _dot(q, _mat(kbuf[us].reshape(r16, nst, 8, 128)))[0:8]
            m = jnp.max(s, axis=1, keepdims=True)
            p = jnp.exp(s - m)
            l = jnp.sum(p, axis=1, keepdims=True)
            v_copy(g).wait()
            o = _dot_nt(_rows16(p), _mat(vbuf[us].reshape(r16, nst, 8, 128)))[0:8]
            o = _rows16(jnp.where(mask, o / l, 0.0))
            o_copy(g).wait()
            return acc + _dot(o, _mat(wob[us].reshape(r16, nct, 8, 128)))[0:8]

        acc = lax.fori_loop(0, ng, group, jnp.zeros((8, d_model), F32))
        return jnp.sum(acc, axis=0, keepdims=True)

    def attention2(x):
        tile_c = _TC / 4
        zero = zero_sc[0]
        zero2 = zero_sc[1]

        def same_head_reduce(v, op):
            v = op(v, pltpu.roll(v, 4, axis=0))
            return op(v, pltpu.roll(v, 2, axis=0))

        rev = {"q": [], "never": None}
        sclk = {"x": None, "n": 0, "t": 0, "base": None}

        def tick(idx, cycles):
            if not sclk["on"]:
                return idx
            if sclk["x"] is None:
                sclk["x"] = idx + zero
            elif sclk["base"] is not idx:
                sclk["x"] = sclk["x"] + (idx - sclk["base"])
            sclk["base"] = idx
            while sclk["n"] < sclk["t"] - _CL0:
                x = sclk["x"]
                sclk["x"] = (x + zero2) if sclk["n"] % 2 else (x ^ zero2)
                sclk["n"] += 1
            sclk["t"] += cycles
            return sclk["x"]

        def tile_dots(lhs, buf, u, c, ntile):
            t = None
            for k in range(ntile):
                l = lhs[k]
                if u is None:
                    w = buf[k * 8:(k + 1) * 8, c].reshape(64, 128)
                else:
                    w = buf[tick(u, _CLN), k * 8:(k + 1) * 8, c].reshape(64, 128)
                for _ in range(_RPT):
                    if rev["q"]:
                        l = jnp.where(rev["never"], pltpu.bitcast(rev["q"].pop(0), U32), l)
                d = _dot(_bf(l), _bf(w))[0:8]
                t = d if t is None else t + d
                yield t

        def task_q(u, par):
            odd_row = (_iota((8, _UW), 0) & 1) == 1
            mask = (_iota((8, _UW), 1) >= _DH) == odd_row
            for c in range(_KT):
                yy = [y_sc[:, _cols(k)] for k in range(nct)]
                for t in tile_dots(yy, wqb, None, u * _KT + c, nct):
                    yield tile_c, 0, None
                t = jnp.where(mask[:, _cols(c)], t * qs_sc[...], 0.0)
                w = pltpu.bitcast(jnp.concatenate([t, t], axis=0).astype(BF16), U32)
                for a in range(_NA):
                    pltpu.store(q_sc[par].at[a, :, _cols(c)], w, mask=_iota((8, 128), 0) == a)
                yield 0.0, 0, t

        def task_s(u, par):
            s = [None] * nj
            for a in range(_NA):
                q = [q_sc[par][a, :, _cols(k)] for k in range(_KT)]
                for j in range(nj):
                    for d in tile_dots(q, kbuf, u, a * nj + j, _KT):
                        yield tile_c, 0, None
                    s[j] = d if a == 0 else s[j] + d
                    z = s[j]
                    if a == _NA - 1:
                        z = mrun = s[j] if j == 0 else jnp.maximum(mrun, s[j])
                    yield 0.0, 0, (z if _TOKS and (j + 1) % _TOKS == 0 else None)
            m = jnp.max(same_head_reduce(mrun, jnp.maximum), axis=1, keepdims=True)
            lrun = None
            for j in range(nj):
                p = jnp.exp2(s[j] - m)
                p_sc[par][:, _cols(j)] = p
                lrun = p if lrun is None else lrun + p
            l_sc[par][...] = lrun
            yield 0.0, _SMLAT, lrun

        def task_x(u, par, nx):
            ox = None
            for st in range(nx):
                a, j = divmod(st, nj)
                t = _dot_nt(_rows16(p_sc[par][:, _cols(j)]),
                            _bf(vbuf[tick(u, 2 * _KT * _CLN), :, st].reshape(_UW // 2, 128)))[0:8]
                ox = t if j == 0 else ox + t
                if j == nj - 1 or st == nx - 1:
                    ox_sc[par][a] = ox
                yield 2 * _KT * tile_c, 0, ox[:, (_KT - 1) * 128:]

        def reduce_o(par, nx):
            row, lane = _iota((8, _UW), 0), _iota((8, _UW), 1)
            head_ok = (lane >= _DH) == ((row & 1) == 1)
            l = jnp.sum(same_head_reduce(l_sc[par][...], jnp.add), axis=1, keepdims=True)
            parts = [jnp.sum(acc_sc[par][_cols(c), :].T, axis=0, keepdims=True)
                     for c in range(_KT)]
            o = jnp.concatenate(parts, axis=1)
            if nx:
                o = o + ox_sc[par][0]
            for a in range(1, -(-nx // nj)):
                o = jnp.where(row >= 2 * a, ox_sc[par][a], o)
            nrow = 2 * max(1, -(-nx // nj))
            return jnp.where(head_ok & (row < nrow), o * (1.0 / l), 0.0)

        def task_o(u, o8):
            o16 = [pltpu.bitcast(_rows16(o8[:, _cols(k)]), U32) for k in range(_KT)]
            for c in range(nct):
                for t in tile_dots(o16, wob, u, c, _KT):
                    yield tile_c, 0, None
                t = t + out_sc[:, _cols(c)]
                out_sc[:, _cols(c)] = t
                yield 0.0, 0, t

        def pv_steps(u, par, nx, tokens, never, clock):
            br = 16 * _BLK
            for b in range(_UW // br):
                h = (b * br) // _DH
                acc = None
                for st in range(nx, nst):
                    a, j = divmod(st, nj)
                    r = 2 * a + h
                    pb = jnp.broadcast_to(p_sc[par][r:r + 1, _cols(j)], (8, 128))
                    for z in tokens():
                        pb = jnp.where(never, z, pb)
                    v = _bf(vbuf[u, b * _BLK:(b + 1) * _BLK, st].reshape(br // 2, 128)).astype(F32)
                    t = v.reshape(br // 8, 8, 128) * pb[None]
                    acc = t if acc is None else acc + t
                    nrev = _REV0 if clock["v"] < _REVT else _REV
                    if nrev and ((st - nx + 1) % nrev == 0 or st == nst - 1):
                        rev["q"] += [acc[i] for i in range(br // 8)]
                    if st == nst - 1:
                        acc_sc[par][b * br:(b + 1) * br, :] = acc.reshape(br, 128)
                    yield _VC * _BLK

        def chain_gens(*gens):
            for g in gens:
                yield from g

        def stage(u, par, nx, nx_prev, do_s=True, do_q=True, order=_ORD):
            never = _iota((8, 128), 1) < zero
            o8 = reduce_o(1 - par, nx_prev)
            pending = [(_RTOK + 100 * c, o8[:, _cols(c)]) for c in range(_KT)]
            um1 = max(u - 1, 0) if isinstance(u, int) else jnp.maximum(u - 1, 0)
            tasks = {"o": task_o(um1, o8), "x": task_x(u, par, nx)}
            if do_s:
                tasks["s"] = task_s(u + 1, 1 - par)
            if do_q:
                tasks["q"] = task_q(u + 2, par)
            mx = chain_gens(*[tasks[k] for k in order if k in tasks])
            clock = {"v": 0.0, "m": 0.0}

            def tokens():
                ready = [z for (t, z) in pending if t <= clock["v"]]
                pending[:] = [(t, z) for (t, z) in pending if t > clock["v"]]
                return ready

            def mx_until(tv):
                while clock["m"] <= tv:
                    try:
                        cm, lat, z = next(mx)
                    except StopIteration:
                        return
                    clock["m"] += cm
                    if z is not None:
                        pending.append((max(clock["m"] + _LAG + lat, _MINT), z))

            rev["never"] = never
            sclk.update(x=None, n=0, t=0, base=None, on=bool(_CLN))
            mx_until(_LEAD)
            for c in pv_steps(u, par, nx, tokens, never, clock):
                clock["v"] += c
                mx_until(clock["v"] + _LEAD)
            rev["q"] = []
            mx_until(1e9)
            sclk["on"] = False

        def region(tag, fn):
            with jax.named_scope("st%02d" % tag):
                pl.when(zero < tag + 1)(fn)

        sclk["on"] = False
        with jax.named_scope("pro"):
            xc, v = _center(x)
            y_sc[...] = pltpu.bitcast(jnp.broadcast_to(xc, (16, d_model)).astype(BF16), U32)
            qs_sc[...] = jnp.broadcast_to(lax.rsqrt(v + _EPS) * (scale * _LOG2E), (8, 128))
            for _ in chain_gens(task_q(0, 0), task_s(0, 0), task_q(1, 1)):
                pass

        if _LOOP:
            def body(i, c):
                region(0, lambda: stage(2 * i, 0, _XM, _XM))
                region(1, lambda: stage(2 * i + 1, 1, _XM, _XM))
                return c
            lax.fori_loop(0, (_NU - 2) // 2, body, 0)
        else:
            for u in range(_NU - 2):
                region(u, functools.partial(stage, u, u % 2, _XM, _XM))
        region(_NU - 2, lambda: stage(_NU - 2, 0, _XP, _XM, do_q=False))
        last = lambda: stage(_NU - 1, 1, _XL, _XP, do_s=False, do_q=False, order=_ORDL)
        if _MRG:
            last()
        else:
            region(_NU - 1, last)
        for _ in task_o(_NU - 1, reduce_o(1, _XL)):
            pass
        return jnp.sum(out_sc[...], axis=0, keepdims=True)

    def mixer(x, first):
        xc, v = _center(x)
        mc = jnp.mean(xc, axis=-1, keepdims=True)
        r1 = lax.rsqrt(v + _EPS)
        r2 = lax.rsqrt(r1 * r1 * (v - mc * mc) + _EPS)
        row = _iota((16, d_model), 0)
        lhs = jnp.where(row < 8, jnp.broadcast_to(xc, (16, d_model)), 1.0).astype(BF16)
        if first:
            w3_copy.wait()
        h = _dot(lhs, _mat(w3b[...]))
        h = (h[0:8] - mc * h[8:16]) * (r1 * r2)
        h = jax.nn.gelu(h, approximate=True)
        h2 = None
        for i, (r0, nr) in enumerate(w4_rows if first else [(0, d_ff)]):
            if first:
                w4_copies[i].wait()
            t = _dot(_rows16(h[:, r0:r0 + nr]), _mat(w4b[r0 // 16:(r0 + nr) // 16]))[0:1]
            h2 = t if h2 is None else h2 + t
        return xc * r1 + h2

    x_copy.wait()
    x = x_ref[...].astype(F32)
    with jax.named_scope("attn1"):
        x = x + attention1(x)
    with jax.named_scope("mix1"):
        x = x + mixer(x, True)
    with jax.named_scope("attn2"):
        x = x + attention2(x)
    with jax.named_scope("mix2"):
        x = x + mixer(x, False)
    o_ref[...] = x.astype(o_ref.dtype)


@jax.jit
def pallas_interleave_layers__sliding_block_cached__mixer_s_mlp__decode_kernel(
    A_x: jax.Array,
    A_k_cache: jax.Array,
    A_v_cache: jax.Array,
    A_wq: jax.Array,
    A_wo: jax.Array,
    B_x: jax.Array,
    B_w1: jax.Array,
    B_w2: jax.Array,
    B_w3: jax.Array,
    B_w4: jax.Array,
):
    b, sq, d_model = A_x.shape
    _, hkv, sk, dh = A_k_cache.shape
    assert b == 1 and sq == 1 and hkv == _HQ and dh == _DH
    win = min(4096, max(256, sk // 4))
    assert win % (128 * _NA) == 0 and (sk - win) % 128 == 0
    d_ff = B_w3.shape[1]

    kt = _tile_view(jnp.swapaxes(A_k_cache, 2, 3).reshape(_NU, _UW, sk))
    vt = _tile_view(jnp.swapaxes(A_v_cache, 2, 3).reshape(_NU, _UW, sk))
    ng = _NU // _GU

    def two(shape, dtype):
        return [pltpu.VMEM(shape, dtype), pltpu.VMEM(shape, dtype)]

    out = pl.pallas_call(
        functools.partial(_kernel, s0=sk - win, win=win),
        out_shape=jax.ShapeDtypeStruct((1, d_model), A_x.dtype),
        in_specs=[pl.BlockSpec(memory_space=pl.ANY)] * 7,
        out_specs=pl.BlockSpec(memory_space=pltpu.VMEM),
        scratch_shapes=[
            pltpu.VMEM((_NU, _UW // 16, win // 128, 8, 128), U32),
            pltpu.VMEM((_NU, _UW // 16, win // 128, 8, 128), U32),
            pltpu.VMEM((d_model // 16, _NU * _KT, 8, 128), U32),
            pltpu.VMEM((_NU, _UW // 16, d_model // 128, 8, 128), U32),
            pltpu.VMEM((d_model // 16, d_ff // 128, 8, 128), U32),
            pltpu.VMEM((d_ff // 16, d_model // 128, 8, 128), U32),
            pltpu.VMEM((1, d_model), A_x.dtype),
            *two((_NA, 8, _UW), U32),
            *two((8, win // _NA), F32),
            *two((_UW, 128), F32),
            *two((_NA, 8, _UW), F32),
            *two((8, 128), F32),
            pltpu.VMEM((8, d_model), U32),
            pltpu.VMEM((8, 128), F32),
            pltpu.VMEM((8, d_model), F32),
            pltpu.SMEM((2,), jnp.int32),
            pltpu.SemaphoreType.DMA((ng,)),
            pltpu.SemaphoreType.DMA((ng,)),
            pltpu.SemaphoreType.DMA((ng,)),
            pltpu.SemaphoreType.DMA((3 + len(_W4C),)),
        ],
        compiler_params=pltpu.CompilerParams(
            vmem_limit_bytes=127 * 1024 * 1024,
            disable_bounds_checks=True, disable_semaphore_checks=True),
        name="interleave_decode",
    )(A_x.reshape(1, d_model), kt, vt, _tile_view(A_wq),
      _tile_view(A_wo.reshape(_NU, _UW, d_model)), _tile_view(B_w3), _tile_view(B_w4))
    return out.reshape(b, sq, d_model)
```

```python
import functools
import os

import jax
import jax.numpy as jnp
from jax import lax
import jax.experimental.pallas as pl
import jax.experimental.pallas.tpu as pltpu

F32 = jnp.float32
BF16 = jnp.bfloat16
U32 = jnp.uint32

_HQ = 32
_DH = 192
_EPS = 1e-5
_LOG2E = 1.4426950408889634
_UW = 2 * _DH
_NU = _HQ // 2
_KT = _UW // 128
_GU = 2
_NA = 4

_E = os.environ.get
_LAG = int(_E("LAG", 180))
_BLK = int(_E("BLK", 2))
_TC = float(_E("TC", 31))
_VC = float(_E("VC", 1.55))
_SMLAT = int(_E("SMLAT", 200))
_RTOK = int(_E("RTOK", 450))
_RSP = int(_E("RSP", 100))
_TOKS = int(_E("TOKS", 1))
_ORD = _E("ORD", "sqox")
_ORDL = _E("ORDL", "xo")
_LEAD = int(_E("LEAD", 0))
_MSL = int(_E("MSL", 100))
_HL = int(_E("HL", 0))
_MINT = int(_E("MINT", 100))
_W4C = [int(t) for t in _E("W4C", "8,3,1").split(",")]
_X0 = int(_E("X0", 2))
_XA = int(_E("XA", 2))
_XB = int(_E("XB", 3))
_XP = int(_E("XP", 2))
_XL = int(_E("XL", 14))
_XS = [_X0] + [(_XA, _XB)[u % 2] for u in range(1, _NU - 2)] + [_XP, _XL]
_KP = int(_E("KP", 15))
_NPRE = 2
_QROW = int(_E("QROW", 0))
_INL = int(_E("INL", 0))


def _bf(x):
    return pltpu.bitcast(x, BF16)


def _tile_view(w):
    *lead, r, c = w.shape
    n = len(lead)
    w = w.reshape(*lead, r // 16, 2, 8, c // 128, 128)
    return w.transpose(*range(n), n, n + 1, n + 3, n + 2, n + 4)


def _mat(x):
    r16, ct = x.shape[0], x.shape[1]
    cols = [x[:, c].reshape(r16 * 8, 128) for c in range(ct)]
    return _bf(cols[0] if ct == 1 else jnp.concatenate(cols, axis=1))


def _dot(a, b):
    return jnp.dot(a, b, preferred_element_type=F32)


def _dot_nt(a, b):
    return lax.dot_general(a, b, (((1,), (1,)), ((), ())), preferred_element_type=F32)


def _iota(shape, axis):
    return lax.broadcasted_iota(jnp.int32, shape, axis)


def _rows16(x8):
    return jnp.concatenate([x8, jnp.zeros_like(x8)], axis=0).astype(BF16)


def _cols(i):
    return slice(i * 128, (i + 1) * 128)


def _center(x):
    xc = x - jnp.mean(x, axis=-1, keepdims=True)
    v = jnp.mean(xc * xc, axis=-1, keepdims=True)
    return xc, v


def _stats(x8):
    n = x8.shape[-1]
    m = jnp.sum(x8, axis=-1, keepdims=True) * (1.0 / n)
    xc = x8 - m
    v = jnp.sum(xc * xc, axis=-1, keepdims=True) * (1.0 / n)
    return m, xc, v


def _all_rows(v):
    for sh in (4, 2, 1):
        v = v + pltpu.roll(v, sh, axis=0)
    return v


def _round(x8):
    return x8.astype(BF16).astype(F32)


class _Retile:
    def __init__(self, src, dst, sem):
        lead = (slice(None),) * (len(dst.shape) - 3)
        self.copies = [
            pltpu.make_async_copy(
                src.at[lead + (a,)],
                dst.at[lead + (slice(None), pl.ds(8 * a, 8))], sem)
            for a in range(2)]

    def start(self):
        for c in self.copies:
            c.start()

    def wait(self):
        for c in self.copies:
            c.wait()


def _kernel(x_hbm, k_hbm, v_hbm, wq_hbm, wo_hbm, w3_hbm, w4_hbm, o_ref,
            kbuf, vbuf, wqb, wob, w3b, w4b, x_ref,
            q_sc, p_sc, acca_sc, accb_sc, y_sc, cs_sc, qs_sc, l_sc, ox_sc, out_sc, zero_sc,
            sem_k, sem_v, sem_o, sem_w, *, s0, win):
    ng = _NU // _GU
    gw = _GU * _UW
    d_model = x_ref.shape[-1]
    d_ff = w3b.shape[1] * 128
    nst = win // 128
    nj = nst // _NA
    nct = d_model // 128
    st0 = s0 // 128

    kb16, vb16, wq16, wo16, w316, w416 = (
        r.bitcast(BF16) for r in (kbuf, vbuf, wqb, wob, w3b, w4b))

    def k_copy(g):
        us = pl.ds(g * _GU, _GU)
        return _Retile(k_hbm.at[us, :, :, pl.ds(st0, nst)], kb16.at[us], sem_k.at[g])

    def v_copy(g):
        us = pl.ds(g * _GU, _GU)
        return _Retile(v_hbm.at[us, :, :, pl.ds(st0, nst)], vb16.at[us], sem_v.at[g])

    def o_copy(g):
        us = pl.ds(g * _GU, _GU)
        return _Retile(wo_hbm.at[us], wo16.at[us], sem_o.at[g])

    wq_copy = _Retile(wq_hbm, wq16, sem_w.at[0])
    w3_copy = _Retile(w3_hbm, w316, sem_w.at[1])
    x_copy = pltpu.make_async_copy(x_hbm, x_ref, sem_w.at[2])
    w4_rows = [(sum(_W4C[:i]) * 128, n * 128) for i, n in enumerate(_W4C)]
    assert sum(_W4C) * 128 == d_ff
    w4_copies = [
        _Retile(w4_hbm.at[pl.ds(r0 // 16, nr // 16)], w416.at[pl.ds(r0 // 16, nr // 16)],
                sem_w.at[3 + i])
        for i, (r0, nr) in enumerate(w4_rows)]

    wq_copy.start()
    x_copy.start()
    for g in range(ng):
        k_copy(g).start()
        v_copy(g).start()
        o_copy(g).start()
    w3_copy.start()
    for c in w4_copies:
        c.start()

    zero_sc[0] = 0
    q_sc[...] = jnp.zeros(q_sc.shape, q_sc.dtype)

    scale = _DH ** -0.5

    def attention1(x):
        _, xc, v = _stats(x)
        y = xc * lax.rsqrt(v + _EPS)
        y_sc[0] = pltpu.bitcast(jnp.concatenate([y, y], axis=0).astype(BF16), U32)
        wq_copy.wait()
        ones = jnp.ones((16, d_model), BF16)
        cs_sc[...] = _dot(ones, _mat(wqb[:, 0:_NPRE * _KT]))[0:8]

        def group(g, acc):
            row_id, lane_id = _iota((8, gw), 0), _iota((8, gw), 1)
            mask = (lane_id >= row_id * _DH) & (lane_id < (row_id + 1) * _DH)
            us = pl.ds(g * _GU, _GU)
            r16 = gw // 16
            q = _dot(_bf(y_sc[0]), _mat(wqb[:, pl.ds(g * (gw // 128), gw // 128)]))[0:8]
            q = _rows16(jnp.where(mask, q * scale, 0.0))
            k_copy(g).wait()
            s = _dot(q, _mat(kbuf[us].reshape(r16, nst, 8, 128)))[0:8]
            m = jnp.max(s, axis=1, keepdims=True)
            p = jnp.exp(s - m)
            l = jnp.sum(p, axis=1, keepdims=True)
            v_copy(g).wait()
            o = _dot_nt(_rows16(p), _mat(vbuf[us].reshape(r16, nst, 8, 128)))[0:8]
            o = _rows16(jnp.where(mask, o / l, 0.0))
            o_copy(g).wait()
            return acc + _dot(o, _mat(wob[us].reshape(r16, nct, 8, 128)))[0:8]

        acc = lax.fori_loop(0, ng, group, jnp.zeros((8, d_model), F32))
        return _all_rows(acc)

    def attention2(x):
        tile_c = _TC / 4
        never = _iota((8, 128), 1) < zero_sc[0]
        acc_sc = (acca_sc, accb_sc)
        nox, parts, started = {}, {}, set()

        zero = zero_sc[0]

        def keep(ref, idx, val, real=True):
            ref[(idx[0] + zero if real else idx[0],) + idx[1:]] = val

        x16 = pltpu.bitcast(jnp.concatenate([x, x], axis=0).astype(BF16), U32)
        mean, xc, v = _stats(x)
        keep(y_sc, (0,), pltpu.bitcast(jnp.concatenate([xc, xc], axis=0).astype(BF16), U32), _KP & 1)
        keep(qs_sc, (0,), jnp.broadcast_to(lax.rsqrt(v + _EPS) * (scale * _LOG2E), (8, 128)), _KP & 1)

        def same_head_reduce(v, op):
            v = op(v, pltpu.roll(v, 4, axis=0))
            return op(v, pltpu.roll(v, 2, axis=0))

        def tile_dots(lhs, tile, ntile):
            t = None
            for k in range(ntile):
                d = _dot(_bf(lhs[k]), _bf(tile(k).reshape(64, 128)))[0:8]
                t = d if t is None else t + d
                yield t

        def head_ok(c):
            return (_iota((8, 128), 1) + c * 128 >= _DH) == ((_iota((8, 128), 0) & 1) == 1)

        def k8(k):
            return slice(k * 8, (k + 1) * 8)

        def task_q(u):
            for c in range(_KT):
                yy = [x16[:, _cols(k)] if u < _NPRE else y_sc[0, :, _cols(k)] for k in range(nct)]
                for t in tile_dots(yy, lambda k: wqb[k8(k), u * _KT + c], nct):
                    yield tile_c, 0, None
                if u < _NPRE:
                    t = t - mean * cs_sc[:, _cols(u * _KT + c)]
                t = jnp.where(head_ok(c), t * qs_sc[0], 0.0)
                w = pltpu.bitcast(jnp.concatenate([t, t], axis=0).astype(BF16), U32)
                for a in range(_NA):
                    if _QROW:
                        q_sc[u, a, a:a + 1, _cols(c)] = w[0:1]
                    else:
                        pltpu.store(q_sc.at[u, a, :, _cols(c)], w, mask=_iota((8, 128), 0) == a)
                yield 0.0, 0, t

        def task_s(u):
            s = [None] * nj
            for a in range(_NA):
                q = [q_sc[u, a, :, _cols(k)] for k in range(_KT)]
                for j in range(nj):
                    for d in tile_dots(q, lambda k: kbuf[u, k8(k), a * nj + j], _KT):
                        yield tile_c, 0, None
                    s[j] = d if a == 0 else s[j] + d
                    z = s[j]
                    if a == _NA - 1:
                        z = mrun = s[j] if j == 0 else jnp.maximum(mrun, s[j])
                    yield 0.0, 0, (z if _TOKS and (j + 1) % _TOKS == 0 else None)
            m = jnp.max(same_head_reduce(mrun, jnp.maximum), axis=1, keepdims=True)
            lrun = None
            for j in range(nj):
                p = jnp.exp2(s[j] - m)
                p_sc[u, :, _cols(j)] = p
                lrun = p if lrun is None else lrun + p
            keep(l_sc, (u,), lrun, _KP & 2)
            yield 0.0, _SMLAT, lrun

        def task_x(u):
            nx = _XS[u]
            nox[u] = -(-nx // nj)
            for st in range(nx):
                a, j = divmod(st, nj)
                t = _dot_nt(_rows16(p_sc[u, :, _cols(j)]),
                            _bf(vbuf[u, :, st].reshape(_UW // 2, 128)))[0:8]
                ox = t if j == 0 else ox + t
                if j == nj - 1 or st == nx - 1:
                    keep(ox_sc, (u, a), ox, _KP & 2)
                yield 2 * _KT * tile_c, 0, ox[:, (_KT - 1) * 128:]

        def lane_sums(u, c):
            t = acc_sc[u % 2][0, _cols(c), :].T
            return jnp.sum(t.reshape(16, 8, 128), axis=0)

        def reduce_o(u):
            row = _iota((8, 128), 0)
            l = jnp.sum(same_head_reduce(l_sc[u], jnp.add), axis=1, keepdims=True)
            linv = jnp.broadcast_to(1.0 / l, (8, 128))
            lswap = pltpu.roll(linv, 1, axis=0)
            pp = parts[u] if _INL else [lane_sums(u, c) for c in range(_KT)]
            res = []
            for c in range(_KT):
                o = pp[c]
                ok = head_ok(c)
                if nox[u]:
                    ox = ox_sc[u, 0, :, _cols(c)]
                    for a in range(1, nox[u]):
                        ox = jnp.where(row >= 2 * a, ox_sc[u, a, :, _cols(c)], ox)
                    o = o + jnp.where(ok & (row < 2 * nox[u]), ox, 0.0)
                res.append(_all_rows(o) * jnp.where(ok, linv, lswap))
            return res

        def task_o(u, o8):
            o16 = [pltpu.bitcast(_rows16(o8[k]), U32) for k in range(_KT)]
            for c in range(nct):
                for t in tile_dots(o16, lambda k: wob[u, k8(k), c], _KT):
                    yield tile_c, 0, None
                if u:
                    t = t + out_sc[0, :, _cols(c)]
                keep(out_sc, (0, slice(None), _cols(c)), t, (_KP & 4) and u + 1 < _NU)
                yield 0.0, 0, t

        pending = []
        clock = {"v": 0.0, "m": -float(_HL)}
        queue = []

        def tokens():
            ready = [z for (t, z) in pending if t <= clock["v"]]
            pending[:] = [(t, z) for (t, z) in pending if t > clock["v"]]
            return ready

        def pv_steps(u):
            br = 16 * _BLK
            parts[u] = []
            for b in range(_UW // br):
                h = (b * br) // _DH
                acc = None
                for st in range(_XS[u], nst):
                    a, j = divmod(st, nj)
                    r = 2 * a + h
                    pb = jnp.broadcast_to(p_sc[u, r:r + 1, _cols(j)], (8, 128))
                    for z in tokens():
                        pb = jnp.where(never, z, pb)
                    v = _bf(vbuf[u, b * _BLK:(b + 1) * _BLK, st].reshape(br // 2, 128)).astype(F32)
                    t = v.reshape(br // 8, 8, 128) * pb[None]
                    acc = t if acc is None else acc + t
                    if st == nst - 1:
                        keep(acc_sc[u % 2], (0, slice(b * br, (b + 1) * br)), acc.reshape(br, 128),
                             (_KP & 8) and u + 1 < _NU)
                        if _INL and (b + 1) * br >= (len(parts[u]) + 1) * 128:
                            part = lane_sums(u, len(parts[u]))
                            parts[u].append(part)
                            pending.append((clock["v"] + _INL, part))
                    yield _VC * _BLK

        def mx_until(tv, need=()):
            while queue and (clock["m"] <= tv or any(q[0] in need for q in queue)):
                try:
                    cm, lat, z = next(queue[0][1])
                except StopIteration:
                    queue.pop(0)
                    continue
                clock["m"] += cm
                if z is not None:
                    pending.append((max(clock["m"] + _LAG + lat, _MINT), z))

        for g in (task_q(0), task_q(1), task_s(0)):
            for _ in g:
                pass
        for u in range(_NU):
            mx_until(-1e9, need=[("s", u), ("x", u - 1)])
            tasks = {"x": task_x(u)}
            if u:
                clock["m"] = max(clock["m"], clock["v"] - _MSL)
                o8 = reduce_o(u - 1)
                pending += [(clock["v"] + _RTOK + _RSP * c, o8[c]) for c in range(_KT)]
                tasks["o"] = task_o(u - 1, o8)
            if u + 1 < _NU:
                tasks["s"] = task_s(u + 1)
            if u + 2 < _NU:
                tasks["q"] = task_q(u + 2)
            key = {"x": u, "o": u - 1, "s": u + 1, "q": u + 2}
            queue += [((k, key[k]), tasks[k]) for k in (_ORD if u + 1 < _NU else _ORDL) if k in tasks]
            mx_until(clock["v"] + _LEAD)
            for c in pv_steps(u):
                clock["v"] += c
                mx_until(clock["v"] + _LEAD)
        mx_until(1e9)
        for _ in task_o(_NU - 1, reduce_o(_NU - 1)):
            pass
        return out_sc[0]

    def mixer(x, first):
        lhs = jnp.concatenate([x, jnp.ones_like(x)], axis=0).astype(BF16)
        m, xc, v = _stats(x)
        mc = jnp.sum(xc, axis=-1, keepdims=True) * (1.0 / d_model)
        r1 = lax.rsqrt(v + _EPS)
        r2 = lax.rsqrt(r1 * r1 * (v - mc * mc) + _EPS)
        if first:
            w3_copy.wait()
        h = _dot(lhs, _mat(w3b[...]))
        h = (h[0:8] - (m + mc) * h[8:16]) * (r1 * r2)
        h = jax.nn.gelu(h, approximate=True)
        h2 = None
        for i, (r0, nr) in enumerate(w4_rows if first else [(0, d_ff)]):
            if first:
                w4_copies[i].wait()
            t = _dot(_rows16(h[:, r0:r0 + nr]), _mat(w4b[r0 // 16:(r0 + nr) // 16]))[0:8]
            h2 = (x + xc * r1) + t if h2 is None else h2 + t
        return h2

    x_copy.wait()
    x = jnp.broadcast_to(x_ref[...].astype(F32), (8, d_model))
    with jax.named_scope("attn1"):
        x = _round(x + attention1(x))
    with jax.named_scope("mix1"):
        x = _round(mixer(x, True))
    with jax.named_scope("attn2"):
        x = _round(x + attention2(x))
    with jax.named_scope("mix2"):
        x = mixer(x, False)
    o_ref[...] = x[0:1].astype(o_ref.dtype)


@jax.jit
def pallas_interleave_layers__sliding_block_cached__mixer_s_mlp__decode_kernel(
    A_x: jax.Array,
    A_k_cache: jax.Array,
    A_v_cache: jax.Array,
    A_wq: jax.Array,
    A_wo: jax.Array,
    B_x: jax.Array,
    B_w1: jax.Array,
    B_w2: jax.Array,
    B_w3: jax.Array,
    B_w4: jax.Array,
):
    b, sq, d_model = A_x.shape
    _, hkv, sk, dh = A_k_cache.shape
    assert b == 1 and sq == 1 and hkv == _HQ and dh == _DH
    win = min(4096, max(256, sk // 4))
    assert win % (128 * _NA) == 0 and (sk - win) % 128 == 0
    d_ff = B_w3.shape[1]

    kt = _tile_view(jnp.swapaxes(A_k_cache, 2, 3).reshape(_NU, _UW, sk))
    vt = _tile_view(jnp.swapaxes(A_v_cache, 2, 3).reshape(_NU, _UW, sk))
    ng = _NU // _GU

    out = pl.pallas_call(
        functools.partial(_kernel, s0=sk - win, win=win),
        out_shape=jax.ShapeDtypeStruct((1, d_model), A_x.dtype),
        in_specs=[pl.BlockSpec(memory_space=pl.ANY)] * 7,
        out_specs=pl.BlockSpec(memory_space=pltpu.VMEM),
        scratch_shapes=[
            pltpu.VMEM((_NU, _UW // 16, win // 128, 8, 128), U32),
            pltpu.VMEM((_NU, _UW // 16, win // 128, 8, 128), U32),
            pltpu.VMEM((d_model // 16, _NU * _KT, 8, 128), U32),
            pltpu.VMEM((_NU, _UW // 16, d_model // 128, 8, 128), U32),
            pltpu.VMEM((d_model // 16, d_ff // 128, 8, 128), U32),
            pltpu.VMEM((d_ff // 16, d_model // 128, 8, 128), U32),
            pltpu.VMEM((1, d_model), A_x.dtype),
            pltpu.VMEM((_NU, _NA, 8, _UW), U32),
            pltpu.VMEM((_NU, 8, win // _NA), F32),
            pltpu.VMEM((1, _UW, 128), F32),
            pltpu.VMEM((1, _UW, 128), F32),
            pltpu.VMEM((1, 8, d_model), U32),
            pltpu.VMEM((8, _NPRE * _UW), F32),
            pltpu.VMEM((1, 8, 128), F32),
            pltpu.VMEM((_NU, 8, 128), F32),
            pltpu.VMEM((_NU, 2, 8, _UW), F32),
            pltpu.VMEM((1, 8, d_model), F32),
            pltpu.SMEM((1,), jnp.int32),
            pltpu.SemaphoreType.DMA((ng,)),
            pltpu.SemaphoreType.DMA((ng,)),
            pltpu.SemaphoreType.DMA((ng,)),
            pltpu.SemaphoreType.DMA((3 + len(_W4C),)),
        ],
        compiler_params=pltpu.CompilerParams(
            vmem_limit_bytes=127 * 1024 * 1024,
            disable_bounds_checks=True, disable_semaphore_checks=True),
        name="interleave_decode",
    )(A_x.reshape(1, d_model), kt, vt, _tile_view(A_wq),
      _tile_view(A_wo.reshape(_NU, _UW, d_model)), _tile_view(B_w3), _tile_view(B_w4))
    return out.reshape(b, sq, d_model)
```

```python
import functools
import os

import jax
import jax.numpy as jnp
from jax import lax
import jax.experimental.pallas as pl
import jax.experimental.pallas.tpu as pltpu

F32 = jnp.float32
BF16 = jnp.bfloat16
U32 = jnp.uint32

_HQ = 32
_DH = 192
_EPS = 1e-5
_LOG2E = 1.4426950408889634
_UW = 2 * _DH
_NU = _HQ // 2
_KT = _UW // 128
_GU = 2
_NA = 4

_E = os.environ.get
_LAG = int(_E("LAG", 160))
_BLK = int(_E("BLK", 2))
_TC = float(_E("TC", 31))
_VC = float(_E("VC", 1.55))
_SMLAT = int(_E("SMLAT", 250))
_RTOK = int(_E("RTOK", 450))
_RSP = int(_E("RSP", 0))
_TOKS = int(_E("TOKS", 1))
_ORD = _E("ORD", "sqxo")
_ORDL = _E("ORDL", "xo")
_LEAD = int(_E("LEAD", 40))
_MSL = int(_E("MSL", 200))
_HL = int(_E("HL", 250))
_MINT = int(_E("MINT", 0))
_W4C = [int(t) for t in _E("W4C", "8,3,1").split(",")]
_X0 = int(_E("X0", 0))
_XA = int(_E("XA", 2))
_XB = int(_E("XB", 2))
_XP = int(_E("XP", 6))
_XL = int(_E("XL", 20))
_X1 = int(_E("X1", 1))
_XC = int(_E("XC", 2))
_XQ = int(_E("XQ", 1))
_XS = [_X0, _X1] + [(_XA, _XB, _XC)[u % 3] for u in range(2, _NU - 3)] + [_XQ, _XP, _XL]
_KP = int(_E("KP", 15))
_NPRE = 2
_NF = int(_E("NF", 8))
_VF = float(_E("VF", 1.05))
_XT = int(_E("XT", 1))
_HS = int(_E("HS", 1))
_NSL = 3
_QROW = int(_E("QROW", 0))
_INL = int(_E("INL", 0))


def _bf(x):
    return pltpu.bitcast(x, BF16)


def _tile_view(w):
    *lead, r, c = w.shape
    n = len(lead)
    w = w.reshape(*lead, r // 16, 2, 8, c // 128, 128)
    return w.transpose(*range(n), n, n + 1, n + 3, n + 2, n + 4)


def _mat(x):
    r16, ct = x.shape[0], x.shape[1]
    cols = [x[:, c].reshape(r16 * 8, 128) for c in range(ct)]
    return _bf(cols[0] if ct == 1 else jnp.concatenate(cols, axis=1))


def _dot(a, b):
    return jnp.dot(a, b, preferred_element_type=F32)


def _dot_nt(a, b):
    return lax.dot_general(a, b, (((1,), (1,)), ((), ())), preferred_element_type=F32)


def _iota(shape, axis):
    return lax.broadcasted_iota(jnp.int32, shape, axis)


def _rows16(x8):
    return jnp.concatenate([x8, jnp.zeros_like(x8)], axis=0).astype(BF16)


def _cols(i):
    return slice(i * 128, (i + 1) * 128)


def _center(x):
    xc = x - jnp.mean(x, axis=-1, keepdims=True)
    v = jnp.mean(xc * xc, axis=-1, keepdims=True)
    return xc, v


def _stats(x8):
    n = x8.shape[-1]
    m = jnp.sum(x8, axis=-1, keepdims=True) * (1.0 / n)
    xc = x8 - m
    v = jnp.sum(xc * xc, axis=-1, keepdims=True) * (1.0 / n)
    return m, xc, v


def _all_rows(v):
    for sh in (4, 2, 1):
        v = v + pltpu.roll(v, sh, axis=0)
    return v


def _round(x8):
    return x8.astype(BF16).astype(F32)


class _Retile:
    def __init__(self, src, dst, sem):
        lead = (slice(None),) * (len(dst.shape) - 3)
        self.copies = [
            pltpu.make_async_copy(
                src.at[lead + (a,)],
                dst.at[lead + (slice(None), pl.ds(8 * a, 8))], sem)
            for a in range(2)]

    def start(self):
        for c in self.copies:
            c.start()

    def wait(self):
        for c in self.copies:
            c.wait()


def _kernel(x_hbm, k_hbm, v_hbm, wq_hbm, wo_hbm, w3_hbm, w4_hbm, o_ref,
            kbuf, vbuf, vfb, wqb, wob, w3b, w4b, x_ref,
            o1_sc, q_sc, p_sc, acca_sc, accb_sc, y_sc, cs_sc, qs_sc, l_sc, ox_sc, out_sc, zero_sc, xs_sc,
            sem_k, sem_v, sem_f, sem_o, sem_w, *, s0, win):
    ng = _NU // _GU
    gw = _GU * _UW
    d_model = x_ref.shape[-1]
    d_ff = w3b.shape[1] * 128
    nst = win // 128
    nj = nst // _NA
    nct = d_model // 128
    st0 = s0 // 128

    nb = nst - _NF
    kb16, vb16, vf16, wq16, wo16, w316, w416 = (
        r.bitcast(BF16) for r in (kbuf, vbuf, vfb, wqb, wob, w3b, w4b))

    def k_copy(g):
        us = pl.ds(g * _GU, _GU)
        return _Retile(k_hbm.at[us, :, :, pl.ds(st0, nst)], kb16.at[us], sem_k.at[g])

    def v_copy(g):
        us = pl.ds(g * _GU, _GU)
        return _Retile(v_hbm.at[us, :, :, pl.ds(st0, nb)], vb16.at[us], sem_v.at[g])

    def f_copy(g):
        us = pl.ds(g * _GU, _GU)
        return _Retile(v_hbm.at[us, :, :, pl.ds(st0 + nb, _NF)], vf16.at[us, :, :, 0], sem_f.at[g])

    wo_copies = [_Retile(wo_hbm.at[pl.ds(g * _GU, _GU)], wo16.at[pl.ds(g * _GU, _GU)], sem_o.at[0])
                 for g in range(ng)]
    wq_copy = _Retile(wq_hbm, wq16, sem_w.at[0])
    w3_copy = _Retile(w3_hbm, w316, sem_w.at[1])
    x_copy = pltpu.make_async_copy(x_hbm, x_ref, sem_w.at[2])
    w4_rows = [(sum(_W4C[:i]) * 128, n * 128) for i, n in enumerate(_W4C)]
    assert sum(_W4C) * 128 == d_ff
    w4_copies = [
        _Retile(w4_hbm.at[pl.ds(r0 // 16, nr // 16)], w416.at[pl.ds(r0 // 16, nr // 16)],
                sem_w.at[3 + i])
        for i, (r0, nr) in enumerate(w4_rows)]

    wq_copy.start()
    x_copy.start()
    for g in range(ng):
        k_copy(g).start()
        v_copy(g).start()
        f_copy(g).start()
    for c in wo_copies:
        c.start()
    w3_copy.start()
    for c in w4_copies:
        c.start()

    zero_sc[0] = 0
    q_sc[...] = jnp.zeros(q_sc.shape, q_sc.dtype)

    scale = _DH ** -0.5

    def ph(u):
        return _NU - 1 - u

    for u in range(_NU):
        xs_sc[ph(u)] = _XS[u] * _KT

    def attention1(x):
        _, xc, v = _stats(x)
        y = xc * lax.rsqrt(v + _EPS)
        y_sc[0] = pltpu.bitcast(jnp.concatenate([y, y], axis=0).astype(BF16), U32)
        wq_copy.wait()
        ones = jnp.ones((16, d_model), BF16)
        cs_sc[...] = _dot(ones, _mat(wqb[:, (_NU - _NPRE) * _KT:]))[0:8]

        def group(g, carry):
            row_id, lane_id = _iota((8, gw), 0), _iota((8, gw), 1)
            mask = (lane_id >= row_id * _DH) & (lane_id < (row_id + 1) * _DH)
            us = pl.ds(g * _GU, _GU)
            r16 = gw // 16
            q = _dot(_bf(y_sc[0]), _mat(wqb[:, pl.ds(g * (gw // 128), gw // 128)]))[0:8]
            q = _rows16(jnp.where(mask, q * scale, 0.0))
            k_copy(g).wait()
            s = _dot(q, _mat(kbuf[us].reshape(r16, nst, 8, 128)))[0:8]
            m = jnp.max(s, axis=1, keepdims=True)
            p = jnp.exp(s - m)
            l = jnp.sum(p, axis=1, keepdims=True)
            v_copy(g).wait()
            f_copy(g).wait()
            o = (_dot_nt(_rows16(p[:, :nb * 128]), _mat(vbuf[us].reshape(r16, nb, 8, 128)))
                 + _dot_nt(_rows16(p[:, nb * 128:]),
                           _mat(vfb[us, :, :, 0].reshape(r16, _NF, 8, 128))))[0:8]
            o1_sc[g] = pltpu.bitcast(_rows16(jnp.where(mask, o / l, 0.0)), U32)

            def widen(i, c):
                u, r = g * _GU + i // (_UW // 16), i % (_UW // 16)
                w = _bf(vfb[u, r, :, 0].reshape(_NF * 8, 128)).astype(F32)
                vfb[u, r] = pltpu.bitcast(w, U32).reshape(_NF, 2, 8, 128)
                return c

            lax.fori_loop(0, r16, widen, 0)

            if _XT:
                for i in range(_GU):
                    u = g * _GU + i

                    def flip(n, c, u=u):
                        rows = pl.ds((n % _KT) * 8, 8)
                        w = _bf(vbuf[u, rows, n // _KT].reshape(64, 128)).astype(F32)
                        w = pltpu.bitcast(w.T.astype(BF16), U32)
                        vbuf[u, rows, n // _KT] = w.reshape(8, 8, 128)
                        return c

                    lax.fori_loop(0, xs_sc[u], flip, 0)
            return carry

        lax.fori_loop(0, ng, group, 0)
        for c in wo_copies:
            c.wait()
        o = _bf(jnp.concatenate([o1_sc[g] for g in range(ng)], axis=1))
        return _all_rows(_dot(o, _mat(wob[...].reshape(_NU * _UW // 16, nct, 8, 128)))[0:8])

    def attention2(x):
        tile_c = _TC / 4
        never = _iota((8, 128), 1) < zero_sc[0]
        acc_sc = (acca_sc, accb_sc)
        nox, parts, started = {}, {}, set()

        zero = zero_sc[0]

        def keep(ref, idx, val, real=True):
            ref[(idx[0] + zero if real else idx[0],) + idx[1:]] = val

        x16 = pltpu.bitcast(jnp.concatenate([x, x], axis=0).astype(BF16), U32)
        mean, xc, v = _stats(x)
        keep(y_sc, (0,), pltpu.bitcast(jnp.concatenate([xc, xc], axis=0).astype(BF16), U32), _KP & 1)
        keep(qs_sc, (0,), jnp.broadcast_to(lax.rsqrt(v + _EPS) * (scale * _LOG2E), (8, 128)), _KP & 1)

        def same_head_reduce(v, op):
            v = op(v, pltpu.roll(v, 4, axis=0))
            return op(v, pltpu.roll(v, 2, axis=0))

        def tile_dots(lhs, tile, ntile):
            t = None
            for k in range(ntile):
                d = _dot(_bf(lhs[k]), _bf(tile(k).reshape(64, 128)))[0:8]
                t = d if t is None else t + d
                yield t

        def head_ok(c):
            return (_iota((8, 128), 1) + c * 128 >= _DH) == ((_iota((8, 128), 0) & 1) == 1)

        def k8(k):
            return slice(k * 8, (k + 1) * 8)

        def task_q(u):
            for c in range(_KT):
                yy = [x16[:, _cols(k)] if u < _NPRE else y_sc[0, :, _cols(k)] for k in range(nct)]
                for t in tile_dots(yy, lambda k: wqb[k8(k), ph(u) * _KT + c], nct):
                    yield tile_c, 0, None
                if u < _NPRE:
                    t = t - mean * cs_sc[:, _cols((ph(u) - _NU + _NPRE) * _KT + c)]
                t = jnp.where(head_ok(c), t if u < _NPRE else t * qs_sc[0], 0.0)
                w = pltpu.bitcast(jnp.concatenate([t, t], axis=0).astype(BF16), U32)
                for a in range(_NA):
                    if _QROW:
                        q_sc[u % _NSL, a, a:a + 1, _cols(c)] = w[0:1]
                    else:
                        pltpu.store(q_sc.at[u % _NSL, a, :, _cols(c)], w, mask=_iota((8, 128), 0) == a)
                yield 0.0, 0, t

        def task_s(u, head=None):
            slot = u % _NSL if head != 1 else _NSL
            s = [None] * nj
            for a in range(_NA):
                q = [q_sc[u % _NSL, a, :, _cols(k)] for k in range(_KT)]
                if head == 0:
                    pieces = [(q[0], slice(0, 8)), (q[1][:, 0:64], slice(8, 12))]
                elif head == 1:
                    pieces = [(q[1][:, 64:128], slice(12, 16)), (q[2], slice(16, 24))]
                else:
                    pieces = [(q[k], k8(k)) for k in range(_KT)]
                for j in range(nj):
                    t = None
                    for l, rows in pieces:
                        nr = rows.stop - rows.start
                        w = kbuf[ph(u), rows, a * nj + j].reshape(nr * 8, 128)
                        d = _dot(_bf(l), _bf(w))[0:8]
                        t = d if t is None else t + d
                        yield tile_c * nr / 8, 0, None
                    s[j] = t if a == 0 else s[j] + t
                    z = s[j]
                    if a == _NA - 1:
                        z = mrun = s[j] if j == 0 else jnp.maximum(mrun, s[j])
                    yield 0.0, 0, (z if _TOKS and (j + 1) % _TOKS == 0 else None)
            m = jnp.max(same_head_reduce(mrun, jnp.maximum), axis=1, keepdims=True)
            lrun = None
            for j in range(nj):
                e = s[j] - m
                p = jnp.exp2(e * qs_sc[0] if u < _NPRE else e)
                p_sc[slot, :, _cols(j)] = p
                lrun = p if lrun is None else lrun + p
            if head == 1:
                lrun = jnp.where((_iota((8, 128), 0) & 1) == 1, lrun, l_sc[u % _NSL])
            keep(l_sc, (u % _NSL,), lrun, _KP & 2)
            yield 0.0, _SMLAT, lrun

        def task_x(u):
            nx = _XS[u]
            nox[u] = -(-nx // nj)
            for st in range(nx):
                a, j = divmod(st, nj)
                p16 = _rows16(p_sc[u % _NSL, :, _cols(j)])
                if _XT:
                    t = jnp.concatenate(
                        [_dot(p16, _bf(vbuf[ph(u), k8(k), st].reshape(64, 128)))[0:8]
                         for k in range(_KT)], axis=1)
                else:
                    t = _dot_nt(p16, _bf(vbuf[ph(u), :, st].reshape(_UW // 2, 128)))[0:8]
                ox = t if j == 0 else ox + t
                if j == nj - 1 or st == nx - 1:
                    keep(ox_sc, (u % _NSL, a), ox, _KP & 2)
                yield (1 if _XT else 2) * _KT * tile_c, 0, ox[:, (_KT - 1) * 128:]

        def lane_sums(u, c):
            t = acc_sc[u % 2][0, _cols(c), :].T
            return jnp.sum(t.reshape(16, 8, 128), axis=0)

        def reduce_o(u):
            row = _iota((8, 128), 0)
            l = jnp.sum(same_head_reduce(l_sc[u % _NSL], jnp.add), axis=1, keepdims=True)
            linv = jnp.broadcast_to(1.0 / l, (8, 128))
            lswap = pltpu.roll(linv, 1, axis=0)
            pp = parts[u] if _INL else [lane_sums(u, c) for c in range(_KT)]
            res = []
            for c in range(_KT):
                o = pp[c]
                ok = head_ok(c)
                if nox[u]:
                    ox = ox_sc[u % _NSL, 0, :, _cols(c)]
                    for a in range(1, nox[u]):
                        ox = jnp.where(row >= 2 * a, ox_sc[u % _NSL, a, :, _cols(c)], ox)
                    o = o + jnp.where(ok & (row < 2 * nox[u]), ox, 0.0)
                res.append(_all_rows(o) * jnp.where(ok, linv, lswap))
            return res

        def task_o(u, o8):
            o16 = [pltpu.bitcast(_rows16(o8[k]), U32) for k in range(_KT)]
            for c in range(nct):
                for t in tile_dots(o16, lambda k: wob[ph(u), k8(k), c], _KT):
                    yield tile_c, 0, None
                if u:
                    t = t + out_sc[0, :, _cols(c)]
                keep(out_sc, (0, slice(None), _cols(c)), t, (_KP & 4) and u + 1 < _NU)
                yield 0.0, 0, t

        pending = []
        clock = {"v": 0.0, "m": -float(_HL)}
        queue = []

        def tokens():
            ready = [z for (t, z) in pending if t <= clock["v"]]
            pending[:] = [(t, z) for (t, z) in pending if t > clock["v"]]
            return ready

        def pv_steps(u):
            br = 16 * _BLK
            parts[u] = []
            for b in range(_UW // br):
                h = (b * br) // _DH
                acc = None
                if _HS and u == 0 and h == 1:
                    mx_until(-1e9, need=[("s1", 0)])
                n16 = nb - _XS[u]
                order = sorted(range(_XS[u], nst), key=lambda st: (
                    (st - _XS[u] + 0.5) / n16 if st < nb else (st - nb + 0.5) / _NF))
                for st in order:
                    a, j = divmod(st, nj)
                    r = 2 * a + h
                    slot = _NSL if (_HS and u == 0 and h == 1) else u % _NSL
                    pb = jnp.broadcast_to(p_sc[slot, r:r + 1, _cols(j)], (8, 128))
                    for z in tokens():
                        pb = jnp.where(never, z, pb)
                    rows = slice(b * _BLK, (b + 1) * _BLK)
                    if st < nb:
                        v = _bf(vbuf[ph(u), rows, st].reshape(br // 2, 128)).astype(F32)
                    else:
                        v = pltpu.bitcast(vfb[ph(u), rows, st - nb].reshape(br, 128), F32)
                    t = v.reshape(br // 8, 8, 128) * pb[None]
                    acc = t if acc is None else acc + t
                    if st == order[-1]:
                        keep(acc_sc[u % 2], (0, slice(b * br, (b + 1) * br)), acc.reshape(br, 128),
                             (_KP & 8) and u + 1 < _NU)
                        if _INL and (b + 1) * br >= (len(parts[u]) + 1) * 128:
                            part = lane_sums(u, len(parts[u]))
                            parts[u].append(part)
                            pending.append((clock["v"] + _INL, part))
                    yield (_VC if st < nb else _VF) * _BLK

        def mx_until(tv, need=()):
            while queue and (clock["m"] <= tv or any(q[0] in need for q in queue)):
                try:
                    cm, lat, z = next(queue[0][1])
                except StopIteration:
                    queue.pop(0)
                    continue
                clock["m"] += cm
                if z is not None:
                    pending.append((max(clock["m"] + _LAG + lat, _MINT), z))

        for g in (task_q(0), task_q(1), task_s(0, 0 if _HS else None)):
            for _ in g:
                pass
        if _HS:
            assert _XS[0] == 0
            queue.append((("s1", 0), task_s(0, 1)))
        for u in range(_NU):
            mx_until(-1e9, need=[("s", u), ("x", u - 1)])
            tasks = {"x": task_x(u)}
            if u:
                clock["m"] = max(clock["m"], clock["v"] - _MSL)
                o8 = reduce_o(u - 1)
                pending += [(clock["v"] + _RTOK + _RSP * c, o8[c]) for c in range(_KT)]
                tasks["o"] = task_o(u - 1, o8)
            if u + 1 < _NU:
                tasks["s"] = task_s(u + 1)
            if u + 2 < _NU:
                tasks["q"] = task_q(u + 2)
            key = {"x": u, "o": u - 1, "s": u + 1, "q": u + 2}
            queue += [((k, key[k]), tasks[k]) for k in (_ORD if u + 1 < _NU else _ORDL) if k in tasks]
            mx_until(clock["v"] + _LEAD)
            for c in pv_steps(u):
                clock["v"] += c
                mx_until(clock["v"] + _LEAD)
        mx_until(1e9)
        for _ in task_o(_NU - 1, reduce_o(_NU - 1)):
            pass
        return out_sc[0]

    def mixer(x, first):
        lhs = jnp.concatenate([x, jnp.ones_like(x)], axis=0).astype(BF16)
        m, xc, v = _stats(x)
        mc = jnp.sum(xc, axis=-1, keepdims=True) * (1.0 / d_model)
        r1 = lax.rsqrt(v + _EPS)
        r2 = lax.rsqrt(r1 * r1 * (v - mc * mc) + _EPS)
        if first:
            w3_copy.wait()
        h = _dot(lhs, _mat(w3b[...]))
        h = (h[0:8] - (m + mc) * h[8:16]) * (r1 * r2)
        h = jax.nn.gelu(h, approximate=True)
        h2 = None
        for i, (r0, nr) in enumerate(w4_rows if first else [(0, d_ff)]):
            if first:
                w4_copies[i].wait()
            t = _dot(_rows16(h[:, r0:r0 + nr]), _mat(w4b[r0 // 16:(r0 + nr) // 16]))[0:8]
            h2 = (x + xc * r1) + t if h2 is None else h2 + t
        return h2

    x_copy.wait()
    x = jnp.broadcast_to(x_ref[...].astype(F32), (8, d_model))
    with jax.named_scope("attn1"):
        x = _round(x + attention1(x))
    with jax.named_scope("mix1"):
        x = _round(mixer(x, True))
    with jax.named_scope("attn2"):
        x = _round(x + attention2(x))
    with jax.named_scope("mix2"):
        x = mixer(x, False)
    o_ref[...] = x[0:1].astype(o_ref.dtype)


@jax.jit
def pallas_interleave_layers__sliding_block_cached__mixer_s_mlp__decode_kernel(
    A_x: jax.Array,
    A_k_cache: jax.Array,
    A_v_cache: jax.Array,
    A_wq: jax.Array,
    A_wo: jax.Array,
    B_x: jax.Array,
    B_w1: jax.Array,
    B_w2: jax.Array,
    B_w3: jax.Array,
    B_w4: jax.Array,
):
    b, sq, d_model = A_x.shape
    _, hkv, sk, dh = A_k_cache.shape
    assert b == 1 and sq == 1 and hkv == _HQ and dh == _DH
    win = min(4096, max(256, sk // 4))
    assert win % (128 * _NA) == 0 and (sk - win) % 128 == 0
    d_ff = B_w3.shape[1]

    kt = _tile_view(jnp.swapaxes(A_k_cache, 2, 3).reshape(_NU, _UW, sk))
    vt = _tile_view(jnp.swapaxes(A_v_cache, 2, 3).reshape(_NU, _UW, sk))
    ng = _NU // _GU

    out = pl.pallas_call(
        functools.partial(_kernel, s0=sk - win, win=win),
        out_shape=jax.ShapeDtypeStruct((1, d_model), A_x.dtype),
        in_specs=[pl.BlockSpec(memory_space=pl.ANY)] * 7,
        out_specs=pl.BlockSpec(memory_space=pltpu.VMEM),
        scratch_shapes=[
            pltpu.VMEM((_NU, _UW // 16, win // 128, 8, 128), U32),
            pltpu.VMEM((_NU, _UW // 16, win // 128 - _NF, 8, 128), U32),
            pltpu.VMEM((_NU, _UW // 16, _NF, 2, 8, 128), U32),
            pltpu.VMEM((d_model // 16, _NU * _KT, 8, 128), U32),
            pltpu.VMEM((_NU, _UW // 16, d_model // 128, 8, 128), U32),
            pltpu.VMEM((d_model // 16, d_ff // 128, 8, 128), U32),
            pltpu.VMEM((d_ff // 16, d_model // 128, 8, 128), U32),
            pltpu.VMEM((1, d_model), A_x.dtype),
            pltpu.VMEM((ng, 8, _GU * _UW), U32),
            pltpu.VMEM((_NSL, _NA, 8, _UW), U32),
            pltpu.VMEM((_NSL + 1, 8, win // _NA), F32),
            pltpu.VMEM((1, _UW, 128), F32),
            pltpu.VMEM((1, _UW, 128), F32),
            pltpu.VMEM((1, 8, d_model), U32),
            pltpu.VMEM((8, _NPRE * _UW), F32),
            pltpu.VMEM((1, 8, 128), F32),
            pltpu.VMEM((_NSL, 8, 128), F32),
            pltpu.VMEM((_NSL, _NA - 1, 8, _UW), F32),
            pltpu.VMEM((1, 8, d_model), F32),
            pltpu.SMEM((1,), jnp.int32),
            pltpu.SMEM((_NU,), jnp.int32),
            pltpu.SemaphoreType.DMA((ng,)),
            pltpu.SemaphoreType.DMA((ng,)),
            pltpu.SemaphoreType.DMA((ng,)),
            pltpu.SemaphoreType.DMA((1,)),
            pltpu.SemaphoreType.DMA((3 + len(_W4C),)),
        ],
        compiler_params=pltpu.CompilerParams(
            vmem_limit_bytes=128 * 1024 * 1024,
            disable_bounds_checks=True, disable_semaphore_checks=True),
        name="interleave_decode",
    )(A_x.reshape(1, d_model), kt, vt, _tile_view(A_wq),
      _tile_view(A_wo.reshape(_NU, _UW, d_model)), _tile_view(B_w3), _tile_view(B_w4))
    return out.reshape(b, sq, d_model)
```

```python
import functools

import jax
import jax.numpy as jnp
from jax import lax
import jax.experimental.pallas as pl
import jax.experimental.pallas.tpu as pltpu

F32 = jnp.float32
BF16 = jnp.bfloat16
U32 = jnp.uint32

_HQ = 32
_DH = 192
_EPS = 1e-5
_LOG2E = 1.4426950408889634
_UW = 2 * _DH
_NU = _HQ // 2
_KT = _UW // 128
_GU = 2
_NA = 4
_W4C = (8, 3, 1)

_NF = 8
_XS = (0, 1) + (2,) * (_NU - 5) + (1, 6, 20)
_BLK = 2
_NPRE = 2
_NSL = 3

_TILE_C = 31.0 / 4
_VC = 1.55
_VF = 1.05
_LAG = 160
_LEAD = 40
_SMLAT = 400
_RTOK = 400
_MSL = 200
_HL = 250
_MINT = 50


def _bf(x):
    return pltpu.bitcast(x, BF16)


def _tile_view(w):
    *lead, r, c = w.shape
    n = len(lead)
    w = w.reshape(*lead, r // 16, 2, 8, c // 128, 128)
    return w.transpose(*range(n), n, n + 1, n + 3, n + 2, n + 4)


def _mat(x):
    r16, ct = x.shape[0], x.shape[1]
    cols = [x[:, c].reshape(r16 * 8, 128) for c in range(ct)]
    return _bf(cols[0] if ct == 1 else jnp.concatenate(cols, axis=1))


def _dot(a, b):
    return jnp.dot(a, b, preferred_element_type=F32)


def _dot_nt(a, b):
    return lax.dot_general(a, b, (((1,), (1,)), ((), ())), preferred_element_type=F32)


def _iota(shape, axis):
    return lax.broadcasted_iota(jnp.int32, shape, axis)


def _rows16(x8):
    return jnp.concatenate([x8, jnp.zeros_like(x8)], axis=0).astype(BF16)


def _dup16(x8):
    return pltpu.bitcast(jnp.concatenate([x8, x8], axis=0).astype(BF16), U32)


def _cols(i):
    return slice(i * 128, (i + 1) * 128)


def _k8(k):
    return slice(k * 8, (k + 1) * 8)


def _stats(x8):
    n = x8.shape[-1]
    m = jnp.sum(x8, axis=-1, keepdims=True) * (1.0 / n)
    xc = x8 - m
    v = jnp.sum(xc * xc, axis=-1, keepdims=True) * (1.0 / n)
    return m, xc, v


def _all_rows(v):
    for sh in (4, 2, 1):
        v = v + pltpu.roll(v, sh, axis=0)
    return v


def _round(x8):
    return x8.astype(BF16).astype(F32)


def _ph(u):
    return _NU - 1 - u


class _Retile:
    def __init__(self, src, dst, sem):
        lead = (slice(None),) * (len(dst.shape) - 3)
        self.copies = [
            pltpu.make_async_copy(
                src.at[lead + (a,)],
                dst.at[lead + (slice(None), pl.ds(8 * a, 8))], sem)
            for a in range(2)]

    def start(self):
        for c in self.copies:
            c.start()

    def wait(self):
        for c in self.copies:
            c.wait()


def _kernel(x_hbm, k_hbm, v_hbm, wq_hbm, wo_hbm, w3_hbm, w4_hbm, o_ref,
            kb16, vb16, vf16, wq16, wo16, w316, w416, x_ref,
            o1_sc, q_sc, p_sc, acca_sc, accb_sc, y_sc, cs_sc, qs_sc, l_sc, ox_sc, out_sc,
            zero_sc, sem_k, sem_v, sem_f, sem_o, sem_w, *, s0, win):
    ng = _NU // _GU
    gw = _GU * _UW
    d_model = x_ref.shape[-1]
    d_ff = w316.shape[1] * 128
    nst = win // 128
    nj = nst // _NA
    nct = d_model // 128
    st0 = s0 // 128
    nb = nst - _NF
    scale = _DH ** -0.5

    kbuf, vbuf, vfb, wqb, wob, w3b, w4b = (
        r.bitcast(U32) for r in (kb16, vb16, vf16, wq16, wo16, w316, w416))

    def k_copy(g):
        us = pl.ds(g * _GU, _GU)
        return _Retile(k_hbm.at[us, :, :, pl.ds(st0, nst)], kb16.at[us], sem_k.at[g])

    def v_copy(g):
        us = pl.ds(g * _GU, _GU)
        return _Retile(v_hbm.at[us, :, :, pl.ds(st0, nb)], vb16.at[us], sem_v.at[g])

    def f_copy(g):
        us = pl.ds(g * _GU, _GU)
        return _Retile(v_hbm.at[us, :, :, pl.ds(st0 + nb, _NF)], vf16.at[us, :, :, 0],
                       sem_f.at[g])

    wo_copies = [
        _Retile(wo_hbm.at[pl.ds(g * _GU, _GU)], wo16.at[pl.ds(g * _GU, _GU)], sem_o.at[0])
        for g in range(ng)]
    wq_copy = _Retile(wq_hbm, wq16, sem_w.at[0])
    w3_copy = _Retile(w3_hbm, w316, sem_w.at[1])
    x_copy = pltpu.make_async_copy(x_hbm, x_ref, sem_w.at[2])
    w4_rows = [(sum(_W4C[:i]) * 128, n * 128) for i, n in enumerate(_W4C)]
    w4_copies = [
        _Retile(w4_hbm.at[pl.ds(r0 // 16, nr // 16)], w416.at[pl.ds(r0 // 16, nr // 16)],
                sem_w.at[3 + i])
        for i, (r0, nr) in enumerate(w4_rows)]

    wq_copy.start()
    x_copy.start()
    for g in range(ng):
        k_copy(g).start()
        v_copy(g).start()
        f_copy(g).start()
    for c in wo_copies:
        c.start()
    w3_copy.start()
    for c in w4_copies:
        c.start()

    zero_sc[0] = 0
    for r in (q_sc, acca_sc, accb_sc, qs_sc, l_sc, ox_sc, out_sc):
        r[...] = jnp.zeros(r.shape, r.dtype)

    def attention1(x):
        _, xc, v = _stats(x)
        y16 = _dup16(xc * lax.rsqrt(v + _EPS))
        for k in range(nct):
            y_sc[k] = y16[:, _cols(k)]
        wq_copy.wait()
        ones = jnp.ones((16, d_model), BF16)
        cs_sc[...] = _dot(ones, _mat(wqb[:, (_NU - _NPRE) * _KT:]))[0:8]

        def group(g, carry):
            row_id, lane_id = _iota((8, gw), 0), _iota((8, gw), 1)
            mask = (lane_id >= row_id * _DH) & (lane_id < (row_id + 1) * _DH)
            us = pl.ds(g * _GU, _GU)
            r16 = gw // 16
            y = _bf(jnp.concatenate([y_sc[k] for k in range(nct)], axis=1))
            q = _dot(y, _mat(wqb[:, pl.ds(g * (gw // 128), gw // 128)]))[0:8]
            q = _rows16(jnp.where(mask, q * scale, 0.0))
            k_copy(g).wait()
            s = _dot(q, _mat(kbuf[us].reshape(r16, nst, 8, 128)))[0:8]
            m = jnp.max(s, axis=1, keepdims=True)
            p = jnp.exp(s - m)
            l = jnp.sum(p, axis=1, keepdims=True)
            v_copy(g).wait()
            f_copy(g).wait()
            o = (_dot_nt(_rows16(p[:, :nb * 128]), _mat(vbuf[us].reshape(r16, nb, 8, 128)))
                 + _dot_nt(_rows16(p[:, nb * 128:]),
                           _mat(vfb[us, :, :, 0].reshape(r16, _NF, 8, 128))))[0:8]
            o1_sc[g] = pltpu.bitcast(_rows16(jnp.where(mask, o / l, 0.0)), U32)

            def widen(i, c):
                u, r = g * _GU + i // (_UW // 16), i % (_UW // 16)
                w = _bf(vfb[u, r, :, 0].reshape(_NF * 8, 128)).astype(F32)
                vf16[u, r] = _bf(w).reshape(_NF, 2, 16, 128)
                return c

            lax.fori_loop(0, r16, widen, 0)

            for i in range(_GU):
                u = g * _GU + i

                def flip(n, c, u=u):
                    rows = pl.ds((n % _KT) * 8, 8)
                    st = jnp.minimum(n // _KT, nb - 1)
                    w = _bf(vbuf[u, rows, st].reshape(64, 128)).astype(F32)
                    vb16[u, rows, st] = w.T.astype(BF16).reshape(8, 16, 128)
                    return c

                ntile = sum(jnp.where(u == _ph(uu), _XS[uu] * _KT, 0) for uu in range(_NU))
                lax.fori_loop(0, ntile, flip, 0)
            return carry

        lax.fori_loop(0, ng, group, 0)
        for c in wo_copies:
            c.wait()
        o = _bf(jnp.concatenate([o1_sc[g] for g in range(ng)], axis=1))
        return _all_rows(_dot(o, _mat(wob[...].reshape(_NU * _UW // 16, nct, 8, 128)))[0:8])

    def attention2(x):
        zero = zero_sc[0]
        never = _iota((8, 128), 1) < zero
        acc_sc = (acca_sc, accb_sc)
        br = 16 * _BLK

        def keep(ref, idx, val):
            ref[(jnp.clip(idx[0] + zero, 0, ref.shape[0] - 1),) + idx[1:]] = val

        x16 = _dup16(x)
        mean, xc, v = _stats(x)
        xc16 = _dup16(xc)
        for k in range(nct):
            y_sc[k] = xc16[:, _cols(k)]
        qs_sc[...] = jnp.broadcast_to(lax.rsqrt(v + _EPS) * (scale * _LOG2E), (8, 128))

        def same_head_reduce(v, op):
            v = op(v, pltpu.roll(v, 4, axis=0))
            return op(v, pltpu.roll(v, 2, axis=0))

        def head_ok(c):
            return (_iota((8, 128), 1) + c * 128 >= _DH) == ((_iota((8, 128), 0) & 1) == 1)

        def tile_dots(lhs, tile, ntile):
            t = None
            for k in range(ntile):
                d = _dot(_bf(lhs[k]), _bf(tile(k).reshape(64, 128)))[0:8]
                t = d if t is None else t + d
                yield t

        def task_q(u):
            for c in range(_KT):
                yy = [x16[:, _cols(k)] if u < _NPRE else y_sc[k] for k in range(nct)]
                for t in tile_dots(yy, lambda k: wqb[_k8(k), _ph(u) * _KT + c], nct):
                    yield _TILE_C, 0, None
                if u < _NPRE:
                    t = t - mean * cs_sc[:, _cols((_ph(u) - _NU + _NPRE) * _KT + c)]
                else:
                    t = t * qs_sc[...]
                t = jnp.where(head_ok(c), t, 0.0)
                w = _dup16(t)
                for a in range(_NA):
                    pltpu.store(q_sc.at[u % _NSL, a, :, _cols(c)], w,
                                mask=_iota((8, 128), 0) == a)
                yield 0.0, 0, t

        def task_s(u, head=None):
            slot = u % _NSL if head != 1 else _NSL
            s = [None] * nj
            for a in range(_NA):
                q = [q_sc[u % _NSL, a, :, _cols(k)] for k in range(_KT)]
                if head == 0:
                    pieces = [(q[0], slice(0, 8)), (q[1][:, 0:64], slice(8, 12))]
                elif head == 1:
                    pieces = [(q[1][:, 64:128], slice(12, 16)), (q[2], slice(16, 24))]
                else:
                    pieces = [(q[k], _k8(k)) for k in range(_KT)]
                for j in range(nj):
                    t = None
                    for l, rows in pieces:
                        nr = rows.stop - rows.start
                        w = kbuf[_ph(u), rows, a * nj + j].reshape(nr * 8, 128)
                        d = _dot(_bf(l), _bf(w))[0:8]
                        t = d if t is None else t + d
                        yield _TILE_C * nr / 8, 0, None
                    s[j] = t if a == 0 else s[j] + t
                    z = s[j]
                    if a == _NA - 1:
                        z = mrun = s[j] if j == 0 else jnp.maximum(mrun, s[j])
                    yield 0.0, 0, z
            m = jnp.max(same_head_reduce(mrun, jnp.maximum), axis=1, keepdims=True)
            lrun = None
            for j in range(nj):
                e = s[j] - m
                p = jnp.exp2(e * qs_sc[...] if u < _NPRE else e)
                p_sc[slot, :, _cols(j)] = p
                lrun = p if lrun is None else lrun + p
            if head == 1:
                lrun = jnp.where((_iota((8, 128), 0) & 1) == 1, lrun, l_sc[u % _NSL])
            keep(l_sc, (u % _NSL,), lrun)
            yield 0.0, _SMLAT, lrun

        def task_x(u):
            for st in range(_XS[u]):
                a, j = divmod(st, nj)
                p16 = _rows16(p_sc[u % _NSL, :, _cols(j)])
                t = jnp.concatenate(
                    [_dot(p16, _bf(vbuf[_ph(u), _k8(k), st].reshape(64, 128)))[0:8]
                     for k in range(_KT)], axis=1)
                ox = t if j == 0 else ox + t
                if j == nj - 1 or st == _XS[u] - 1:
                    keep(ox_sc, (u % _NSL, a), ox)
                yield _KT * _TILE_C, 0, ox[:, (_KT - 1) * 128:]

        def reduce_o(u):
            row = _iota((8, 128), 0)
            nox = -(-_XS[u] // nj)
            nbk = 128 // br
            l = jnp.sum(same_head_reduce(l_sc[u % _NSL], jnp.add), axis=1, keepdims=True)
            linv = jnp.broadcast_to(1.0 / l, (8, 128))
            lswap = pltpu.roll(linv, 1, axis=0)
            parts = []
            for c in range(_KT):
                t = acc_sc[u % 2][c * nbk:(c + 1) * nbk].reshape(128, 128).T
                parts.append(jnp.sum(t.reshape(16, 8, 128), axis=0))
            res = []
            for c in range(_KT):
                o = parts[c]
                ok = head_ok(c)
                if nox:
                    ox = ox_sc[u % _NSL, 0, :, _cols(c)]
                    for a in range(1, nox):
                        ox = jnp.where(row >= 2 * a, ox_sc[u % _NSL, a, :, _cols(c)], ox)
                    o = o + jnp.where(ok & (row < 2 * nox), ox, 0.0)
                res.append(_all_rows(o) * jnp.where(ok, linv, lswap))
            return res

        def task_o(u, o8):
            o16 = [pltpu.bitcast(_rows16(o8[k]), U32) for k in range(_KT)]
            for c in range(nct):
                for t in tile_dots(o16, lambda k: wob[_ph(u), _k8(k), c], _KT):
                    yield _TILE_C, 0, None
                if u:
                    t = t + out_sc[c]
                if u + 1 < _NU:
                    keep(out_sc, (c,), t)
                else:
                    out_sc[c] = t
                yield 0.0, 0, t

        pending = []
        clock = {"v": 0.0, "m": -float(_HL)}
        queue = []

        def tokens():
            ready = [z for (t, z) in pending if t <= clock["v"]]
            pending[:] = [(t, z) for (t, z) in pending if t > clock["v"]]
            return ready

        def mx_until(tv, need=()):
            while queue and (clock["m"] <= tv or any(q[0] in need for q in queue)):
                try:
                    cm, lat, z = next(queue[0][1])
                except StopIteration:
                    queue.pop(0)
                    continue
                clock["m"] += cm
                if z is not None:
                    pending.append((max(clock["m"] + _LAG + lat, _MINT), z))

        def pv_steps(u):
            n16 = nb - _XS[u]
            order = sorted(range(_XS[u], nst), key=lambda st: (
                (st - _XS[u] + 0.5) / n16 if st < nb else (st - nb + 0.5) / _NF))
            for b in range(_UW // br):
                h = (b * br) // _DH
                slot = u % _NSL
                if u == 0 and h == 1:
                    mx_until(-1e9, need=[("s1", 0)])
                    slot = _NSL
                rows = slice(b * _BLK, (b + 1) * _BLK)
                acc = None
                for st in order:
                    a, j = divmod(st, nj)
                    r = 2 * a + h
                    pb = jnp.broadcast_to(p_sc[slot, r:r + 1, _cols(j)], (8, 128))
                    for z in tokens():
                        pb = jnp.where(never, z, pb)
                    if st < nb:
                        v = _bf(vbuf[_ph(u), rows, st].reshape(br // 2, 128)).astype(F32)
                    else:
                        v = pltpu.bitcast(vfb[_ph(u), rows, st - nb].reshape(br, 128), F32)
                    t = v.reshape(br // 8, 8, 128) * pb[None]
                    acc = t if acc is None else acc + t
                    if st == order[-1]:
                        if u + 1 < _NU:
                            keep(acc_sc[u % 2], (b,), acc.reshape(br, 128))
                        else:
                            acc_sc[u % 2][b] = acc.reshape(br, 128)
                    yield (_VC if st < nb else _VF) * _BLK

        for g in (task_q(0), task_q(1), task_s(0, 0)):
            for _ in g:
                pass
        queue.append((("s1", 0), task_s(0, 1)))
        for u in range(_NU):
            mx_until(-1e9, need=[("s", u), ("x", u - 1)])
            if u:
                clock["m"] = max(clock["m"], clock["v"] - _MSL)
                o8 = reduce_o(u - 1)
                pending += [(clock["v"] + _RTOK, o8[c]) for c in range(_KT)]
            if u + 1 < _NU:
                queue.append((("s", u + 1), task_s(u + 1)))
            if u + 2 < _NU:
                queue.append((("q", u + 2), task_q(u + 2)))
            queue.append((("x", u), task_x(u)))
            if u:
                queue.append((("o", u - 1), task_o(u - 1, o8)))
            mx_until(clock["v"] + _LEAD)
            for c in pv_steps(u):
                clock["v"] += c
                mx_until(clock["v"] + _LEAD)
        mx_until(1e9)
        for _ in task_o(_NU - 1, reduce_o(_NU - 1)):
            pass
        return jnp.concatenate([out_sc[c] for c in range(nct)], axis=1)

    def mixer(x, first):
        lhs = jnp.concatenate([x, jnp.ones_like(x)], axis=0).astype(BF16)
        m, xc, v = _stats(x)
        mc = jnp.sum(xc, axis=-1, keepdims=True) * (1.0 / d_model)
        r1 = lax.rsqrt(v + _EPS)
        r2 = lax.rsqrt(r1 * r1 * (v - mc * mc) + _EPS)
        if first:
            w3_copy.wait()
        h = _dot(lhs, _mat(w3b[...]))
        h = (h[0:8] - (m + mc) * h[8:16]) * (r1 * r2)
        h = jax.nn.gelu(h, approximate=True)
        out = x + xc * r1
        for i, (r0, nr) in enumerate(w4_rows if first else [(0, d_ff)]):
            if first:
                w4_copies[i].wait()
            out = out + _dot(_rows16(h[:, r0:r0 + nr]),
                             _mat(w4b[r0 // 16:(r0 + nr) // 16]))[0:8]
        return out

    x_copy.wait()
    x = jnp.broadcast_to(x_ref[...].astype(F32), (8, d_model))
    x = _round(x + attention1(x))
    x = _round(mixer(x, True))
    x = _round(x + attention2(x))
    x = mixer(x, False)
    o_ref[...] = x[0:1].astype(o_ref.dtype)


@jax.jit
def pallas_interleave_layers__sliding_block_cached__mixer_s_mlp__decode_kernel(
    A_x: jax.Array,
    A_k_cache: jax.Array,
    A_v_cache: jax.Array,
    A_wq: jax.Array,
    A_wo: jax.Array,
    B_x: jax.Array,
    B_w1: jax.Array,
    B_w2: jax.Array,
    B_w3: jax.Array,
    B_w4: jax.Array,
):
    b, sq, d_model = A_x.shape
    _, hkv, sk, dh = A_k_cache.shape
    assert b == 1 and sq == 1 and hkv == _HQ and dh == _DH
    win = min(4096, max(256, sk // 4))
    nst = win // 128
    d_ff = B_w3.shape[1]
    assert win % (128 * _NA) == 0 and (sk - win) % 128 == 0
    assert _XS[0] == 0 and max(_XS) < nst - _NF and sum(_W4C) * 128 == d_ff

    kt = _tile_view(jnp.swapaxes(A_k_cache, 2, 3).reshape(_NU, _UW, sk))
    vt = _tile_view(jnp.swapaxes(A_v_cache, 2, 3).reshape(_NU, _UW, sk))
    ng = _NU // _GU
    br = 16 * _BLK

    out = pl.pallas_call(
        functools.partial(_kernel, s0=sk - win, win=win),
        out_shape=jax.ShapeDtypeStruct((1, d_model), A_x.dtype),
        in_specs=[pl.BlockSpec(memory_space=pl.ANY)] * 7,
        out_specs=pl.BlockSpec(memory_space=pltpu.VMEM),
        scratch_shapes=[
            pltpu.VMEM((_NU, _UW // 16, nst, 16, 128), BF16),
            pltpu.VMEM((_NU, _UW // 16, nst - _NF, 16, 128), BF16),
            pltpu.VMEM((_NU, _UW // 16, _NF, 2, 16, 128), BF16),
            pltpu.VMEM((d_model // 16, _NU * _KT, 16, 128), BF16),
            pltpu.VMEM((_NU, _UW // 16, d_model // 128, 16, 128), BF16),
            pltpu.VMEM((d_model // 16, d_ff // 128, 16, 128), BF16),
            pltpu.VMEM((d_ff // 16, d_model // 128, 16, 128), BF16),
            pltpu.VMEM((1, d_model), A_x.dtype),
            pltpu.VMEM((ng, 8, _GU * _UW), U32),
            pltpu.VMEM((_NSL, _NA, 8, _UW), U32),
            pltpu.VMEM((_NSL + 1, 8, win // _NA), F32),
            pltpu.VMEM((_UW // br, br, 128), F32),
            pltpu.VMEM((_UW // br, br, 128), F32),
            pltpu.VMEM((d_model // 128, 8, 128), U32),
            pltpu.VMEM((8, _NPRE * _UW), F32),
            pltpu.VMEM((8, 128), F32),
            pltpu.VMEM((_NSL, 8, 128), F32),
            pltpu.VMEM((_NSL, _NA - 1, 8, _UW), F32),
            pltpu.VMEM((d_model // 128, 8, 128), F32),
            pltpu.SMEM((1,), jnp.int32),
            pltpu.SemaphoreType.DMA((ng,)),
            pltpu.SemaphoreType.DMA((ng,)),
            pltpu.SemaphoreType.DMA((ng,)),
            pltpu.SemaphoreType.DMA((1,)),
            pltpu.SemaphoreType.DMA((3 + len(_W4C),)),
        ],
        compiler_params=pltpu.CompilerParams(
            vmem_limit_bytes=128 * 1024 * 1024,
            disable_bounds_checks=True, disable_semaphore_checks=True),
        name="interleave_decode",
    )(A_x.reshape(1, d_model), kt, vt, _tile_view(A_wq),
      _tile_view(A_wo.reshape(_NU, _UW, d_model)), _tile_view(B_w3), _tile_view(B_w4))
    return out.reshape(b, sq, d_model)
```

```python
import functools

import jax
import jax.numpy as jnp
from jax import lax
import jax.experimental.pallas as pl
import jax.experimental.pallas.tpu as pltpu

F32 = jnp.float32
BF16 = jnp.bfloat16
U32 = jnp.uint32

_HQ = 32
_DH = 192
_EPS = 1e-5
_LOG2E = 1.4426950408889634
_UW = 2 * _DH
_NU = _HQ // 2
_KT = _UW // 128
_GU = 2
_NA = 4
_W4C = (7, 3, 1, 1)

_NF = 8
_XS = (0, 0, 4, 4, 5, 2, 2, 3, 2, 3, 2, 2, 2, 1, 6, 20)
_BLK = 2
_NHS = 2
_VQ = (4, 5, 6)
_NV4 = 6
_NSL = 3

_TILE_C = 31.0 / 4
_VC = 1.57
_VF = 1.08
_VQC = 4.7
_VQ0 = 300
_VQR = 8
_LAG = 180
_LEAD = 40
_SMLAT = 250
_RTOK = 400
_MSL = 200


def _bf(x):
    return pltpu.bitcast(x, BF16)


def _tile_view(w):
    *lead, r, c = w.shape
    n = len(lead)
    w = w.reshape(*lead, r // 16, 2, 8, c // 128, 128)
    return w.transpose(*range(n), n, n + 1, n + 3, n + 2, n + 4)


def _mat(x):
    r16, ct = x.shape[0], x.shape[1]
    cols = [x[:, c].reshape(r16 * 8, 128) for c in range(ct)]
    return _bf(cols[0] if ct == 1 else jnp.concatenate(cols, axis=1))


def _dot(a, b):
    return jnp.dot(a, b, preferred_element_type=F32)


def _dot_nt(a, b):
    return lax.dot_general(a, b, (((1,), (1,)), ((), ())), preferred_element_type=F32)


def _iota(shape, axis):
    return lax.broadcasted_iota(jnp.int32, shape, axis)


def _rows16(x8):
    return jnp.concatenate([x8, jnp.zeros_like(x8)], axis=0).astype(BF16)


def _dup16(x8):
    return pltpu.bitcast(jnp.concatenate([x8, x8], axis=0).astype(BF16), U32)


def _cols(i):
    return slice(i * 128, (i + 1) * 128)


def _k8(k):
    return slice(k * 8, (k + 1) * 8)


def _stats(x8):
    n = x8.shape[-1]
    m = jnp.sum(x8, axis=-1, keepdims=True) * (1.0 / n)
    xc = x8 - m
    v = jnp.sum(xc * xc, axis=-1, keepdims=True) * (1.0 / n)
    return m, xc, v


def _all_rows(v):
    for sh in (4, 2, 1):
        v = v + pltpu.roll(v, sh, axis=0)
    return v


def _down(x8):
    return jnp.concatenate([x8] * 16, axis=0).T


def _round(x8):
    return x8.astype(BF16).astype(F32)


def _ph(u):
    return _NU - 1 - u


class _Retile:
    def __init__(self, src, dst, sem):
        lead = (slice(None),) * (len(dst.shape) - 3)
        self.copies = [
            pltpu.make_async_copy(
                src.at[lead + (a,)],
                dst.at[lead + (slice(None), pl.ds(8 * a, 8))], sem)
            for a in range(2)]

    def start(self):
        for c in self.copies:
            c.start()

    def wait(self):
        for c in self.copies:
            c.wait()


def _kernel(x_hbm, k_hbm, v_hbm, wq_hbm, wo_hbm, w3_hbm, w4_hbm, o_ref,
            kb16, vb16, vf16, wq16, wo16, w316, w416, x_ref,
            qv_sc, q_sc, p_sc, acca_sc, accb_sc, y_sc, cs_sc, qs_sc, l_sc, ox_sc, out_sc,
            zero_sc, sem_k, sem_v, sem_f, sem_o, sem_w, *, s0, win):
    ng = _NU // _GU
    gw = _GU * _UW
    d_model = x_ref.shape[-1]
    d_ff = w316.shape[1] * 128
    nst = win // 128
    nj = nst // _NA
    nct = d_model // 128
    st0 = s0 // 128
    nb = nst - _NF
    scale = _DH ** -0.5

    kbuf, vbuf, vfb, wqb, wob, w3b, w4b = (
        r.bitcast(U32) for r in (kb16, vb16, vf16, wq16, wo16, w316, w416))

    vff = vf16.bitcast(F32)

    def k_copy(g):
        us = pl.ds(g * _GU, _GU)
        return _Retile(k_hbm.at[us, :, :, pl.ds(st0, nst)], kb16.at[us], sem_k.at[g])

    def v_copy(g):
        us = pl.ds(g * _GU, _GU)
        return _Retile(v_hbm.at[us, :, :, pl.ds(st0, nb)], vb16.at[us], sem_v.at[g])

    def f_copy(g):
        us = pl.ds(g * _GU, _GU)
        return _Retile(v_hbm.at[us, :, :, pl.ds(st0 + nb, _NF)], vf16.at[us, :, :, 0],
                       sem_f.at[g])

    wo_copies = [
        _Retile(wo_hbm.at[pl.ds(g * _GU, _GU)], wo16.at[pl.ds(g * _GU, _GU)], sem_o.at[0])
        for g in range(ng)]
    wq_copy = _Retile(wq_hbm, wq16, sem_w.at[0])
    w3_copy = _Retile(w3_hbm, w316, sem_w.at[1])
    x_copy = pltpu.make_async_copy(x_hbm, x_ref, sem_w.at[2])
    w4_rows = [(sum(_W4C[:i]) * 128, n * 128) for i, n in enumerate(_W4C)]
    w4_copies = [
        _Retile(w4_hbm.at[pl.ds(r0 // 16, nr // 16)], w416.at[pl.ds(r0 // 16, nr // 16)],
                sem_w.at[3 + i])
        for i, (r0, nr) in enumerate(w4_rows)]

    wq_copy.start()
    x_copy.start()
    for g in range(ng):
        k_copy(g).start()
        v_copy(g).start()
        f_copy(g).start()
    for c in wo_copies:
        c.start()
    w3_copy.start()
    for c in w4_copies:
        c.start()

    zero_sc[0] = 0
    for r in (qv_sc, q_sc, acca_sc, accb_sc, qs_sc, l_sc, ox_sc, out_sc):
        r[...] = jnp.zeros(r.shape, r.dtype)

    def attention1(x, stats):
        _, xc, v = stats
        y16 = _dup16(xc * lax.rsqrt(v + _EPS))
        for k in range(nct):
            y_sc[k] = y16[:, _cols(k)]
        wq_copy.wait()
        ones = jnp.ones((16, d_model), BF16)
        cs_sc[...] = _dot(ones, _mat(wqb[:, (_NU - _NHS) * _KT:]))[0:8]

        def group(g, carry):
            row_id, lane_id = _iota((8, gw), 0), _iota((8, gw), 1)
            mask = (lane_id >= row_id * _DH) & (lane_id < (row_id + 1) * _DH)
            us = pl.ds(g * _GU, _GU)
            r16 = gw // 16
            y = _bf(jnp.concatenate([y_sc[k] for k in range(nct)], axis=1))
            q = _dot(y, _mat(wqb[:, pl.ds(g * (gw // 128), gw // 128)]))[0:8]
            q = _rows16(jnp.where(mask, q * scale, 0.0))
            k_copy(g).wait()
            s = _dot(q, _mat(kbuf[us].reshape(r16, nst, 8, 128)))[0:8]
            m = jnp.max(s, axis=1, keepdims=True)
            p = jnp.exp(s - m)
            l = jnp.sum(p, axis=1, keepdims=True)
            v_copy(g).wait()
            f_copy(g).wait()
            o = (_dot_nt(_rows16(p[:, :nb * 128]), _mat(vbuf[us].reshape(r16, nb, 8, 128)))
                 + _dot_nt(_rows16(p[:, nb * 128:]),
                           _mat(vfb[us, :, :, 0].reshape(r16, _NF, 8, 128))))[0:8]
            o = pltpu.bitcast(_rows16(jnp.where(mask, o / l, 0.0)), F32)
            for c in range(gw // 128):
                acca_sc[g * (gw // 128) + c] = o[:, _cols(c)]

            def widen(i, c):
                u, r = g * _GU + i // (_UW // 16), i % (_UW // 16)
                w = _bf(vfb[u, r, :, 0].reshape(_NF * 8, 128)).astype(F32)
                vf16[u, r] = _bf(w).reshape(_NF, 2, 16, 128)
                return c

            lax.fori_loop(0, r16, widen, 0)

            for i in range(_GU):
                u = g * _GU + i

                def flip(n, c, u=u):
                    rows = pl.ds((n % _KT) * 8, 8)
                    st = jnp.minimum(n // _KT, nb - 1)
                    w = _bf(vbuf[u, rows, st].reshape(64, 128)).astype(F32)
                    vb16[u, rows, st] = w.T.astype(BF16).reshape(8, 16, 128)
                    return c

                ntile = sum(jnp.where(u == _ph(uu), _XS[uu] * _KT, 0) for uu in range(_NU))
                lax.fori_loop(0, ntile, flip, 0)
            return carry

        lax.fori_loop(0, ng, group, 0)
        for c in wo_copies:
            c.wait()
        o = _bf(jnp.concatenate([acca_sc[c] for c in range(_NU * _KT)], axis=1))
        return _all_rows(_dot(o, _mat(wob[...].reshape(_NU * _UW // 16, nct, 8, 128)))[0:8])

    def attention2(x, stats):
        zero = zero_sc[0]
        never = _iota((8, 128), 1) < zero
        acc_sc = (acca_sc, accb_sc)
        br = 16 * _BLK

        def keep(ref, idx, val):
            n = val.shape[0]
            ref[pl.ds(jnp.clip(idx + zero, 0, ref.shape[0] - n), n)] = val

        x16 = _dup16(x)
        mean, xc, v = stats
        xc16 = _dup16(xc)
        for k in range(nct):
            y_sc[k] = xc16[:, _cols(k)]
        qs_sc[...] = jnp.broadcast_to(lax.rsqrt(v + _EPS) * (scale * _LOG2E), (8, 128))

        def same_head_reduce(v, op):
            v = op(v, pltpu.roll(v, 4, axis=0))
            return op(v, pltpu.roll(v, 2, axis=0))

        def head_ok(c):
            return (_iota((8, 128), 1) + c * 128 >= _DH) == ((_iota((8, 128), 0) & 1) == 1)

        def tile_dots(lhs, tile, ntile):
            t = None
            for k in range(ntile):
                d = _dot(_bf(lhs[k]), _bf(tile(k).reshape(64, 128)))[0:8]
                t = d if t is None else t + d
                yield t

        pending = []
        rev = []
        clock = {"v": float(_VQ0), "m": 0.0}
        queue = []
        owner = {}

        def tokens():
            ready = [z for (t, z) in pending if t <= clock["v"]]
            pending[:] = [(t, z) for (t, z) in pending if t > clock["v"]]
            return ready

        def mx_until(tv, need=()):
            while queue and (clock["m"] <= tv or any(q[0] in need for q in queue)):
                try:
                    cm, lat, z = next(queue[0][1])
                except StopIteration:
                    queue.pop(0)
                    continue
                clock["m"] += cm
                if z is not None:
                    pending.append((clock["m"] + _LAG + lat, z))

        def finish_q(u, c, t):
            if u < _NHS:
                t = t - mean * cs_sc[:, _cols((_ph(u) - _NU + _NHS) * _KT + c)]
            else:
                t = t * qs_sc[...]
            return jnp.where(head_ok(c), t, 0.0)

        def task_q(u):
            owner["q", u % 2] = u
            for c in range(_KT):
                if u in _VQ:
                    t, w = None, qv_sc[_VQ.index(u) * _KT + c]
                else:
                    yy = [x16[:, _cols(k)] if u < _NHS else y_sc[k] for k in range(nct)]
                    for t in tile_dots(yy, lambda k: wqb[_k8(k), _ph(u) * _KT + c], nct):
                        yield _TILE_C, 0, None
                    t = finish_q(u, c, t)
                    w = _dup16(t)
                for a in range(_NA):
                    pltpu.store(q_sc.at[u % 2, a, :, _cols(c)], w,
                                mask=_iota((8, 128), 0) == a)
                if t is not None:
                    yield 0.0, 0, t

        def vq_steps():
            cols = [_down(x[:, _cols(k)]) for k in range(nct)]
            tiles = [(u, c) for u in _VQ for c in range(_KT)]
            acc = {}
            for n in range(d_model // 16):
                k, r = divmod(n, 8)
                xa = cols[k][r * 16:r * 16 + 8] - mean
                xb = cols[k][r * 16 + 8:r * 16 + 16] - mean
                for z in tokens():
                    xa = jnp.where(never, z, xa)
                for u, c in tiles:
                    w = wq16[n, _ph(u) * _KT + c].astype(F32)
                    t = w[0:8] * xa + w[8:16] * xb
                    acc[u, c] = t if n == 0 else acc[u, c] + t
                if (n + 1) % _VQR == 0:
                    rev.extend(acc[uc] for uc in tiles)
                yield _VQC * len(_VQ)
            for i, (u, c) in enumerate(tiles):
                t = finish_q(u, c, _all_rows(acc[u, c]))
                keep(qv_sc, i, _dup16(t)[None])
                pending.append((clock["v"] + 150, t))

        def p_slot(u, h):
            return (u - 1) % _NSL if u < _NHS and h == 1 else u % _NSL

        def task_s(u, head=None):
            slot = p_slot(u, head)
            s = [None] * nj
            for a in range(_NA):
                assert owner["q", u % 2] == u
                q = [q_sc[u % 2, a, :, _cols(k)] for k in range(_KT)]
                if head == 0:
                    pieces = [(q[0], slice(0, 8)), (q[1][:, 0:64], slice(8, 12))]
                elif head == 1:
                    pieces = [(q[1][:, 64:128], slice(12, 16)), (q[2], slice(16, 24))]
                else:
                    pieces = [(q[k], _k8(k)) for k in range(_KT)]
                for j in range(nj):
                    t = None
                    for l, rows in pieces:
                        nr = rows.stop - rows.start
                        w = kbuf[_ph(u), rows, a * nj + j].reshape(nr * 8, 128)
                        if nr == 8:
                            for _ in range(min(len(rev), 2)):
                                l = jnp.where(never, pltpu.bitcast(rev.pop(0), U32), l)
                        d = _dot(_bf(l), _bf(w))[0:8]
                        t = d if t is None else t + d
                        yield _TILE_C * nr / 8, 0, None
                    s[j] = t if a == 0 else s[j] + t
                    z = s[j]
                    if a == _NA - 1:
                        z = mrun = s[j] if j == 0 else jnp.maximum(mrun, s[j])
                    yield 0.0, 0, z
            m = jnp.max(same_head_reduce(mrun, jnp.maximum), axis=1, keepdims=True)
            owner["p", slot] = u
            lrun = None
            for j in range(nj):
                e = s[j] - m
                p = jnp.exp2(e * qs_sc[...] if u < _NHS else e)
                p_sc[slot, :, _cols(j)] = p
                lrun = p if lrun is None else lrun + p
            if head == 1:
                lrun = jnp.where((_iota((8, 128), 0) & 1) == 1, lrun, l_sc[u % _NSL])
            keep(l_sc, u % _NSL, lrun[None])
            yield 0.0, _SMLAT, lrun

        def task_x(u):
            for st in range(_XS[u]):
                a, j = divmod(st, nj)
                assert owner["p", u % _NSL] == u
                p16 = _rows16(p_sc[u % _NSL, :, _cols(j)])
                t = jnp.concatenate(
                    [_dot(p16, _bf(vbuf[_ph(u), _k8(k), st].reshape(64, 128)))[0:8]
                     for k in range(_KT)], axis=1)
                ox = t if j == 0 else ox + t
                if j == nj - 1 or st == _XS[u] - 1:
                    keep(ox_sc, u % _NSL + a, ox[None])
                yield _KT * _TILE_C, 0, ox[:, (_KT - 1) * 128:]

        def reduce_o(u):
            row = _iota((8, 128), 0)
            nox = -(-_XS[u] // nj)
            l = jnp.sum(same_head_reduce(l_sc[u % _NSL], jnp.add), axis=1, keepdims=True)
            linv = jnp.broadcast_to(1.0 / l, (8, 128))
            lswap = pltpu.roll(linv, 1, axis=0)
            parts = []
            for c in range(_KT):
                t = acc_sc[u % 2][c * 16:(c + 1) * 16].reshape(128, 128).T
                parts.append(jnp.sum(t.reshape(16, 8, 128), axis=0))
            res = []
            for c in range(_KT):
                o = parts[c]
                ok = head_ok(c)
                if nox:
                    ox = ox_sc[u % _NSL, :, _cols(c)]
                    for a in range(1, nox):
                        ox = jnp.where(row >= 2 * a, ox_sc[u % _NSL + a, :, _cols(c)], ox)
                    o = o + jnp.where(ok & (row < 2 * nox), ox, 0.0)
                res.append(_all_rows(o) * jnp.where(ok, linv, lswap))
            return res

        def task_o(u, o8):
            o16 = [pltpu.bitcast(_rows16(o8[k]), U32) for k in range(_KT)]
            for c in range(nct):
                for t in tile_dots(o16, lambda k: wob[_ph(u), _k8(k), c], _KT):
                    yield _TILE_C, 0, None
                if u:
                    t = t + out_sc[c]
                if u + 1 < _NU:
                    keep(out_sc, c, t[None])
                else:
                    out_sc[c] = t
                yield 0.0, 0, t

        def pv_steps(u):
            n16 = nb - _XS[u]
            order = sorted(range(_XS[u], nst), key=lambda st: (
                (st - _XS[u] + 0.5) / n16 if st < nb else (st - nb + 0.5) / _NF))
            for b in range(_UW // br):
                h = (b * br) // _DH
                slot = p_slot(u, h)
                if h == 1:
                    mx_until(-1e9, need=[("s1", u)])
                rows = slice(b * _BLK, (b + 1) * _BLK)
                acc = None
                for st in order:
                    a, j = divmod(st, nj)
                    r = 2 * a + h
                    assert owner["p", slot] == u
                    pb = jnp.broadcast_to(p_sc[slot, r:r + 1, _cols(j)], (8, 128))
                    for z in tokens():
                        pb = jnp.where(never, z, pb)
                    if st < nb:
                        v = vb16[_ph(u), rows, st].astype(F32)
                    else:
                        v = vff[_ph(u), rows, st - nb]
                    t = v.reshape(br // 8, 8, 128) * pb[None]
                    acc = t if acc is None else acc + t
                    if st == order[-1]:
                        if u + 1 < _NU:
                            keep(acc_sc[u % 2], b * br // 8, acc)
                        else:
                            acc_sc[u % 2][b * br // 8:(b + 1) * br // 8] = acc
                    yield (_VC if st < nb else _VF) * _BLK

        queue += [(("q", 0), task_q(0)), (("q", 1), task_q(1)),
                  (("s", 0), task_s(0, 0)), (("s1", 0), task_s(0, 1)),
                  (("s", 1), task_s(1, 0)), (("q", 2), task_q(2)), (("s1", 1), task_s(1, 1))]
        mx_until(clock["v"])
        for c in vq_steps():
            clock["v"] += c
            mx_until(clock["v"])
        for u in range(_NU):
            mx_until(-1e9, need=[("s", u), ("x", u - 1)])
            if u:
                clock["m"] = max(clock["m"], clock["v"] - _MSL)
                o8 = reduce_o(u - 1)
                pending += [(clock["v"] + _RTOK, o8[c]) for c in range(_KT)]
                if u + 1 < _NU:
                    queue.append((("s", u + 1), task_s(u + 1)))
                if u + 2 < _NU:
                    queue.append((("q", u + 2), task_q(u + 2)))
                queue.append((("x", u), task_x(u)))
                queue.append((("o", u - 1), task_o(u - 1, o8)))
            mx_until(clock["v"] + _LEAD)
            for c in pv_steps(u):
                clock["v"] += c
                mx_until(clock["v"] + _LEAD)
        mx_until(1e9)
        for _ in task_o(_NU - 1, reduce_o(_NU - 1)):
            pass
        return jnp.concatenate([out_sc[c] for c in range(nct)], axis=1)

    def mixer(x, pivot, first):
        lhs = jnp.concatenate([x, jnp.ones_like(x)], axis=0).astype(BF16)
        d = x - pivot
        s1 = jnp.sum(d, axis=-1, keepdims=True) * (1.0 / d_model)
        s2 = jnp.sum(d * d, axis=-1, keepdims=True) * (1.0 / d_model)
        m = pivot + s1
        v = jnp.maximum(s2 - s1 * s1, 0.0)
        xc = x - m
        mc = s1 - (m - pivot)
        r1 = lax.rsqrt(v + _EPS)
        r2 = lax.rsqrt(r1 * r1 * v + _EPS)
        if first:
            w3_copy.wait()
        h = _dot(lhs, _mat(w3b[...]))
        h = (h[0:8] - (m + mc) * h[8:16]) * (r1 * r2)
        h = jax.nn.gelu(h, approximate=True)
        out = x + xc * r1

        def w4_vpu(cols):
            chunks = list(cols)
            acc = [None] * nct
            for n0 in range(0, len(chunks), 2):
                for r in range(8):
                    for n in chunks[n0:n0 + 2]:
                        hc = cols[n][r * 16:(r + 1) * 16]
                        for c in range(nct):
                            t = w416[n * 8 + r, c].astype(F32) * hc
                            acc[c] = t if acc[c] is None else acc[c] + t
            return jnp.concatenate([_all_rows(a[0:8] + a[8:16]) for a in acc], axis=1)

        def w4_mxu(r0, nr):
            return _dot(_rows16(h[:, r0:r0 + nr]), _mat(w4b[r0 // 16:(r0 + nr) // 16]))[0:8]

        if first:
            cols = {r0 // 128: _down(h[:, r0:r0 + nr]) for r0, nr in w4_rows if nr == 128}
            for i, (r0, nr) in enumerate(w4_rows):
                w4_copies[i].wait()
                if nr == 128:
                    out = out + w4_vpu({r0 // 128: cols[r0 // 128]})
                else:
                    out = out + w4_mxu(r0, nr)
            return out
        part = w4_vpu({n: _down(h[:, _cols(n)]) for n in range(_NV4)})
        for n in range(_NV4, d_ff // 128):
            out = out + w4_mxu(n * 128, 128)
        return out + part

    x_copy.wait()
    x = jnp.broadcast_to(x_ref[...].astype(F32), (8, d_model))
    for first, attention in ((True, attention1), (False, attention2)):
        stats = _stats(x)
        x = mixer(_round(x + attention(x, stats)), stats[0], first)
        x = _round(x) if first else x
    o_ref[...] = x[0:1].astype(o_ref.dtype)


@jax.jit
def pallas_interleave_layers__sliding_block_cached__mixer_s_mlp__decode_kernel(
    A_x: jax.Array,
    A_k_cache: jax.Array,
    A_v_cache: jax.Array,
    A_wq: jax.Array,
    A_wo: jax.Array,
    B_x: jax.Array,
    B_w1: jax.Array,
    B_w2: jax.Array,
    B_w3: jax.Array,
    B_w4: jax.Array,
):
    b, sq, d_model = A_x.shape
    _, hkv, sk, dh = A_k_cache.shape
    assert b == 1 and sq == 1 and hkv == _HQ and dh == _DH
    win = min(4096, max(256, sk // 4))
    nst = win // 128
    d_ff = B_w3.shape[1]
    assert win % (128 * _NA) == 0 and (sk - win) % 128 == 0
    assert (_NU - 1) % _NSL == 0 and max(_XS[:-1]) <= nst // _NA
    assert _XS[-1] <= _NSL * (nst // _NA) and _NHS == 2
    assert not any(_XS[:_NHS]) and max(_XS) < nst - _NF and sum(_W4C) * 128 == d_ff

    kt = _tile_view(jnp.swapaxes(A_k_cache, 2, 3).reshape(_NU, _UW, sk))
    vt = _tile_view(jnp.swapaxes(A_v_cache, 2, 3).reshape(_NU, _UW, sk))
    ng = _NU // _GU

    out = pl.pallas_call(
        functools.partial(_kernel, s0=sk - win, win=win),
        out_shape=jax.ShapeDtypeStruct((1, d_model), A_x.dtype),
        in_specs=[pl.BlockSpec(memory_space=pl.ANY)] * 7,
        out_specs=pl.BlockSpec(memory_space=pltpu.VMEM),
        scratch_shapes=[
            pltpu.VMEM((_NU, _UW // 16, nst, 16, 128), BF16),
            pltpu.VMEM((_NU, _UW // 16, nst - _NF, 16, 128), BF16),
            pltpu.VMEM((_NU, _UW // 16, _NF, 2, 16, 128), BF16),
            pltpu.VMEM((d_model // 16, _NU * _KT, 16, 128), BF16),
            pltpu.VMEM((_NU, _UW // 16, d_model // 128, 16, 128), BF16),
            pltpu.VMEM((d_model // 16, d_ff // 128, 16, 128), BF16),
            pltpu.VMEM((d_ff // 16, d_model // 128, 16, 128), BF16),
            pltpu.VMEM((1, d_model), A_x.dtype),
            pltpu.VMEM((len(_VQ) * _KT, 8, 128), U32),
            pltpu.VMEM((2, _NA, 8, _UW), U32),
            pltpu.VMEM((_NSL, 8, win // _NA), F32),
            pltpu.VMEM((_UW // 8, 8, 128), F32),
            pltpu.VMEM((_UW // 8, 8, 128), F32),
            pltpu.VMEM((d_model // 128, 8, 128), U32),
            pltpu.VMEM((8, _NHS * _UW), F32),
            pltpu.VMEM((8, 128), F32),
            pltpu.VMEM((_NSL, 8, 128), F32),
            pltpu.VMEM((_NSL, 8, _UW), F32),
            pltpu.VMEM((d_model // 128, 8, 128), F32),
            pltpu.SMEM((1,), jnp.int32),
            pltpu.SemaphoreType.DMA((ng,)),
            pltpu.SemaphoreType.DMA((ng,)),
            pltpu.SemaphoreType.DMA((ng,)),
            pltpu.SemaphoreType.DMA((1,)),
            pltpu.SemaphoreType.DMA((3 + len(_W4C),)),
        ],
        compiler_params=pltpu.CompilerParams(
            vmem_limit_bytes=128 * 1024 * 1024,
            disable_bounds_checks=True, disable_semaphore_checks=True),
        name="interleave_decode",
    )(A_x.reshape(1, d_model), kt, vt, _tile_view(A_wq),
      _tile_view(A_wo.reshape(_NU, _UW, d_model)), _tile_view(B_w3), _tile_view(B_w4))
    return out.reshape(b, sq, d_model)
```
